```python
import jax
import jax.numpy as jnp

def _softmax(x, axis=-1):
    return jax.nn.softmax(x, axis=axis)
def _gelu(x):
    return jax.nn.gelu(x, approximate=True)
def _silu(x):
    return jax.nn.silu(x)
def _sigmoid(x):
    return jax.nn.sigmoid(x)
def _layernorm(x, axis=-1, eps=1e-5):
    m = jnp.mean(x, axis=axis, keepdims=True)
    v = jnp.var(x, axis=axis, keepdims=True)
    return (x - m) / jnp.sqrt(v + eps)
def _scatter_add(tgt, idx, src, axis=0):
    return tgt.at[idx].add(src)
def _segment_sum(src, seg, n):
    return jax.ops.segment_sum(src, seg, n)
class _Rng:
    def __init__(self, key):
        self._k = key
    def _next(self):
        self._k, sub = jax.random.split(self._k)
        return sub
    def normal(self, shape):
        return jax.random.normal(self._next(), shape, dtype=jnp.bfloat16)
    def randint(self, lo, hi, shape):
        return jax.random.randint(self._next(), shape, lo, hi, dtype=jnp.int32)
    def uniform(self, shape, lo=0.0, hi=1.0):
        return jax.random.uniform(self._next(), shape, jnp.bfloat16, lo, hi)
    def permutation(self, n):
        return jax.random.permutation(self._next(), n)


kernel_name = 'parallel_sum__ssm_conv_s5__moe_arch_mod__prompt'

def setup_inputs():
    _rng = _Rng(jax.random.key(int.from_bytes(__import__("os").urandom(4), "little")))
    _w = (lambda a: (lambda t: t.astype(jnp.bfloat16) if jnp.issubdtype(t.dtype, jnp.floating) else t)(jnp.asarray(a)))
    def _A_setup():
        B, S, D = 1, 2048, 1024
        P = D
        Lambda_re = -0.5 * jnp.exp((lambda *s: _rng.normal(s) * 0.05)(P))
        Lambda_im = (lambda *s: _rng.normal(s) * 0.05)(P) * 1.0
        B_re = (lambda *s: _rng.normal(s) * 0.05)(P, D) * (D ** -0.5)
        B_im = (lambda *s: _rng.normal(s) * 0.05)(P, D) * (D ** -0.5)
        C_re = (lambda *s: _rng.normal(s) * 0.05)(D, P) * (P ** -0.5)
        C_im = (lambda *s: _rng.normal(s) * 0.05)(D, P) * (P ** -0.5)
        log_dt = (lambda *s: _rng.normal(s) * 0.05)(P) * 0.3 - 2.0
        Dskip = (lambda *s: _rng.normal(s) * 0.05)(D)
        return {
            "x": _w((lambda *s: _rng.normal(s) * 0.05)(B, S, D)),
            "Lambda_re": _w(Lambda_re),
            "Lambda_im": _w(Lambda_im),
            "B_re": _w(B_re),
            "B_im": _w(B_im),
            "C_re": _w(C_re),
            "C_im": _w(C_im),
            "log_dt": _w(log_dt),
            "Dskip": _w(Dskip),
        }
    _A_in = _A_setup()

    def _B_setup():
        B, S, D, F, C = 1, 2048, 1024, 3584, 2
        return {
            "x": _w((lambda *s: _rng.normal(s) * 0.05)(B, S, D)),
            "w_r": _w((lambda *s: _rng.normal(s) * 0.05)(D)),
            "w_gate": _w((lambda *s: _rng.normal(s) * 0.05)(D, F)),
            "w_up": _w((lambda *s: _rng.normal(s) * 0.05)(D, F)),
            "w_down": _w((lambda *s: _rng.normal(s) * 0.05)(F, D)),
        }
    _B_in = _B_setup()

    return {
        "A_x": _A_in["x"],
        "A_Lambda_re": _A_in["Lambda_re"],
        "A_Lambda_im": _A_in["Lambda_im"],
        "A_B_re": _A_in["B_re"],
        "A_B_im": _A_in["B_im"],
        "A_C_re": _A_in["C_re"],
        "A_C_im": _A_in["C_im"],
        "A_log_dt": _A_in["log_dt"],
        "A_Dskip": _A_in["Dskip"],
        "B_x": _B_in["x"],
        "B_w_r": _B_in["w_r"],
        "B_w_gate": _B_in["w_gate"],
        "B_w_up": _B_in["w_up"],
        "B_w_down": _B_in["w_down"],
    }

def reference(A_x, A_Lambda_re, A_Lambda_im, A_B_re, A_B_im, A_C_re, A_C_im, A_log_dt, A_Dskip, B_x, B_w_r, B_w_gate, B_w_up, B_w_down):
    def _A_ref(x, Lambda_re, Lambda_im, B_re, B_im, C_re, C_im, log_dt, Dskip):
        Bsz, L, H = x.shape
        Lam = Lambda_re + 1j * Lambda_im
        Bmat = B_re + 1j * B_im
        Cmat = C_re + 1j * C_im
        dt = jnp.exp(log_dt)
        Lam_bar = jnp.exp(dt * Lam)
        B_bar = ((Lam_bar - 1.0) / Lam)[:, None] * Bmat
        Bu = jnp.einsum("bld,pd->blp", x + 0j, B_bar)
        h = jnp.zeros_like(Bu[:, 0, :])
        hs = []
        for t in range(L):
            h = Lam_bar[None, :] * h + Bu[:, t, :]
            hs.append(h)
        hseq = jnp.stack(hs, 1)
        y = 2.0 * jnp.einsum("blp,dp->bld", hseq, Cmat).real + x * Dskip[None, None, :]
        return y

    def _B_ref(x, w_r, w_gate, w_up, w_down):
        B, S, D = x.shape
        C = 2
        r = x @ w_r
        idx = jnp.argsort(-r, axis=-1)[:, :C]
        idx_e = jnp.repeat(idx.reshape(B, C, 1), D, axis=2)
        x_sel = jnp.take_along_axis(x, idx_e, axis=1)
        g = _silu(x_sel @ w_gate)
        u = x_sel @ w_up
        y = (g * u) @ w_down
        r_sel = _sigmoid(jnp.take_along_axis(r, idx, axis=1))
        y = y * r_sel.reshape(B, C, 1)
        b_off = (jnp.arange(B) * S).reshape(B, 1)
        flat_idx = (idx + b_off).reshape(B * C)
        zero = (x * 0.0).reshape(B * S, D)
        upd = _scatter_add(zero, flat_idx, y.reshape(B * C, D), axis=0)
        return x + upd.reshape(B, S, D)

    x = A_x
    xn = _layernorm(x, axis=-1)
    return x + _A_ref(xn, A_Lambda_re, A_Lambda_im, A_B_re, A_B_im, A_C_re, A_C_im, A_log_dt, A_Dskip) + _B_ref(xn, B_w_r, B_w_gate, B_w_up, B_w_down)
```

```python
import functools

import jax
import jax.numpy as jnp
import jax.experimental.pallas as pl
import jax.experimental.pallas.tpu as pltpu

F32 = jnp.float32
BF16 = jnp.bfloat16
NSEG = 8


def _rb(v):
    return v.astype(BF16).astype(F32)


def _layernorm_rows(x):
    d = x.shape[-1]
    m = jnp.sum(x, axis=-1, keepdims=True) * (1.0 / d)
    xc = x - m
    v = jnp.sum(xc * xc, axis=-1, keepdims=True) * (1.0 / d)
    s = _rb(jnp.sqrt(_rb(_rb(v) + 1e-5)))
    return _rb(_rb(x - _rb(m)) / s)


def _nt(a, b):
    return jax.lax.dot_general(a, b, (((1,), (1,)), ((), ())), preferred_element_type=F32)


def _kernel(x_hbm, lre_ref, lim_ref, bre_hbm, bim_hbm, cre_hbm, cim_hbm, ldt_ref, dsk_ref,
            wr_ref, wg_hbm, wu_hbm, wd_hbm, o_hbm,
            xv, bre, bim, cre, cim, wg, wu, wd, res, bure, buim, hre, him, rsc,
            car, stage, hb, sem_x, sem_b, sem_w, sem_o, *, J, PC):
    KD, S, _ = res.shape
    D = KD * 128
    P = bre.shape[0]
    SEG = S // NSEG
    NB = SEG // J
    T = NSEG * J
    NC = P // PC

    def x_copy(b):
        return pltpu.make_async_copy(
            x_hbm.at[:, pl.ds(b * J, J), :], xv.at[:, pl.ds(b * J, J), :], sem_x.at[b])

    def b_copy(c, src, dst, k):
        return pltpu.make_async_copy(
            src.at[pl.ds(c * PC, PC), :], dst.at[pl.ds(c * PC, PC), :], sem_b.at[2 * c + k])

    w_copies = [pltpu.make_async_copy(s_, d_, sem_w.at[i]) for i, (s_, d_) in enumerate(
        ((cre_hbm, cre), (cim_hbm, cim), (wg_hbm, wg), (wu_hbm, wu), (wd_hbm, wd)))]

    def o_copy(b, slot):
        return pltpu.make_async_copy(
            stage.at[slot], o_hbm.at[:, pl.ds(b * J, J), :], sem_o.at[slot])

    x_copy(0).start()
    for c in range(NC):
        b_copy(c, bre_hbm, bre, 0).start()
        b_copy(c, bim_hbm, bim, 1).start()
    for b in range(1, NB):
        x_copy(b).start()
    for cp in w_copies:
        cp.start()

    lre = lre_ref[...].astype(F32)
    lim = lim_ref[...].astype(F32)
    dt = _rb(jnp.exp(ldt_ref[...].astype(F32)))
    mag = jnp.exp(dt * lre)
    are = mag * jnp.cos(dt * lim)
    aim = mag * jnp.sin(dt * lim)
    den = lre * lre + lim * lim
    kre = ((are - 1.0) * lre + aim * lim) / den
    kim = (aim * lre - (are - 1.0) * lim) / den
    are8 = jnp.broadcast_to(are, (NSEG, P))
    aim8 = jnp.broadcast_to(aim, (NSEG, P))
    dsk = dsk_ref[...].astype(F32)
    wr = wr_ref[...].astype(F32)

    hre[...] = jnp.zeros_like(hre)
    him[...] = jnp.zeros_like(him)

    def p1_block(b, first):
        x_copy(b).wait()
        r0 = pl.multiple_of(b * T, T)
        j0 = pl.multiple_of(b * J, J)
        for s in range(NSEG):
            xs = xv[s, pl.ds(j0, J), :].astype(F32)
            for k in range(KD):
                res[k, pl.ds(r0 + s, J, stride=NSEG), :] = xs[:, k * 128:(k + 1) * 128]
        x = jnp.concatenate([res[k, pl.ds(r0, T), :] for k in range(KD)], axis=1)
        xn = _layernorm_rows(x)
        rs = x + xn + _rb(xn * dsk)
        for k in range(KD):
            res[k, pl.ds(r0, T), :] = rs[:, k * 128:(k + 1) * 128]
        rsc[pl.ds(r0, T), :] = jnp.broadcast_to(
            _rb(jnp.sum(xn * wr, axis=-1, keepdims=True)), (T, 128))
        xb = xn.astype(BF16)
        for c in range(NC):
            cs = slice(c * PC, (c + 1) * PC)
            if first:
                b_copy(c, bre_hbm, bre, 0).wait()
                b_copy(c, bim_hbm, bim, 1).wait()
            ure = _nt(xb, bre[cs, :])
            uim = _nt(xb, bim[cs, :])
            bure[pl.ds(r0, T), cs] = ure
            buim[pl.ds(r0, T), cs] = uim
            ar, ai = are8[:, cs], aim8[:, cs]
            hr, hi = hre[:, cs], him[:, cs]
            for j in range(J):
                js = slice(j * NSEG, (j + 1) * NSEG)
                hr, hi = (ar * hr + ure[js]) - ai * hi, (ar * hi + uim[js]) + ai * hr
            hre[:, cs] = hr
            him[:, cs] = hi

    p1_block(0, True)
    jax.lax.fori_loop(1, NB, lambda b, _: p1_block(b, False), None)

    pr, pi = are8, aim8
    for _ in range(SEG.bit_length() - 1):
        pr, pi = pr * pr - pi * pi, 2.0 * pr * pi
    sub = jax.lax.broadcasted_iota(jnp.int32, (NSEG, P), 0)
    er, ei = hre[...], him[...]
    sh = 1
    while sh < NSEG:
        tr = jnp.where(sub >= sh, pltpu.roll(er, sh, 0), 0.0)
        ti = jnp.where(sub >= sh, pltpu.roll(ei, sh, 0), 0.0)
        er, ei = er + (pr * tr - pi * ti), ei + (pr * ti + pi * tr)
        pr, pi = pr * pr - pi * pi, 2.0 * pr * pi
        sh *= 2
    hre[...] = jnp.where(sub >= 1, pltpu.roll(er, 1, 0), 0.0)
    him[...] = jnp.where(sub >= 1, pltpu.roll(ei, 1, 0), 0.0)

    w_copies[0].wait()
    w_copies[1].wait()

    def c_prep(i, _):
        rows = pl.ds(pl.multiple_of(i * 128, 128), 128)
        cr = cre[rows, :].astype(F32)
        ci = cim[rows, :].astype(F32)
        cre[rows, :] = (2.0 * (cr * kre - ci * kim)).astype(BF16)
        cim[rows, :] = (-2.0 * (cr * kim + ci * kre)).astype(BF16)

    jax.lax.fori_loop(0, D // 128, c_prep, None)

    row = jax.lax.broadcasted_iota(jnp.int32, (S, 128), 0)
    tix = (row % NSEG) * SEG + row // NSEG
    rr = rsc[...]
    m1 = jnp.max(rr)
    t1 = jnp.min(jnp.where(rr == m1, tix, S))
    rr = jnp.where(tix == t1, -jnp.inf, rr)
    m2 = jnp.max(rr)
    t2 = jnp.min(jnp.where((rr == m2) & (tix != t1), tix, S))
    t1 = jnp.clip(t1, 0, S - 1)
    t2 = jnp.clip(t2, 0, S - 1)

    sub16 = jax.lax.broadcasted_iota(jnp.int32, (16, D), 0)

    def pick(t):
        s, j = t // SEG, t % SEG
        g = pl.multiple_of((j // 16) * 16, 16)
        xn = _layernorm_rows(xv[s, pl.ds(g, 16), :].astype(F32))
        return jnp.sum(jnp.where(sub16 == j % 16, xn, 0.0), axis=0, keepdims=True)

    xs = jnp.where(sub16 == 0, pick(t1), jnp.where(sub16 == 1, pick(t2), 0.0)).astype(BF16)
    w_copies[2].wait()
    w_copies[3].wait()
    g = _rb(jnp.dot(xs, wg[...], preferred_element_type=F32))
    u = _rb(jnp.dot(xs, wu[...], preferred_element_type=F32))
    act = (_rb(g * jax.nn.sigmoid(g)) * u).astype(BF16)
    w_copies[4].wait()
    y = jnp.dot(act, wd[...], preferred_element_type=F32)
    for k, (t, m) in enumerate(((t1, m1), (t2, m2))):
        prow = pl.ds((t % SEG) * NSEG + t // SEG, 1)
        gate = jax.nn.sigmoid(jnp.full((1, D), m, F32))
        yk = y[k:k + 1, :] * gate
        for q in range(KD):
            res[q, prow, :] = res[q, prow, :] + yk[:, q * 128:(q + 1) * 128]

    def p2_block(b, _):
        slot = b % 2
        r0 = pl.multiple_of(b * T, T)
        for c in range(NC):
            cs = slice(c * PC, (c + 1) * PC)
            ar, ai = are8[:, cs], aim8[:, cs]
            hr, hi = hre[:, cs], him[:, cs]
            for j in range(0, J, 2):
                rows = pl.ds(pl.multiple_of(r0 + j * NSEG, 16), 16)
                ur, ui = bure[rows, cs], buim[rows, cs]
                hr0, hi0 = (ar * hr + ur[:8]) - ai * hi, (ar * hi + ui[:8]) + ai * hr
                hr, hi = (ar * hr0 + ur[8:]) - ai * hi0, (ar * hi0 + ui[8:]) + ai * hr0
                hb[0, j * NSEG:(j + 2) * NSEG, cs] = jnp.concatenate([hr0, hr], 0).astype(BF16)
                hb[1, j * NSEG:(j + 2) * NSEG, cs] = jnp.concatenate([hi0, hi], 0).astype(BF16)
            hre[:, cs] = hr
            him[:, cs] = hi
        y = _nt(hb[0], cre[...]) + _nt(hb[1], cim[...])
        for k in range(KD):
            car[k] = y[:, k * 128:(k + 1) * 128] + res[k, pl.ds(r0, T), :]

        @pl.when(b >= 2)
        def _():
            o_copy(b - 2, slot).wait()

        for s in range(NSEG):
            stage[slot, s] = jnp.concatenate(
                [car[k, pl.ds(s, J, stride=NSEG), :] for k in range(KD)], axis=1)
        o_copy(b, slot).start()

    jax.lax.fori_loop(0, NB, p2_block, None)
    o_copy(NB - 2, 0).wait()
    o_copy(NB - 1, 1).wait()


@jax.jit
def pallas_parallel_sum__ssm_conv_s5__moe_arch_mod__prompt_kernel(
    A_x: jax.Array,
    A_Lambda_re: jax.Array,
    A_Lambda_im: jax.Array,
    A_B_re: jax.Array,
    A_B_im: jax.Array,
    A_C_re: jax.Array,
    A_C_im: jax.Array,
    A_log_dt: jax.Array,
    A_Dskip: jax.Array,
    B_x: jax.Array,
    B_w_r: jax.Array,
    B_w_gate: jax.Array,
    B_w_up: jax.Array,
    B_w_down: jax.Array,
):
    del B_x
    Bsz, S, D = A_x.shape
    P = A_B_re.shape[0]
    F = B_w_gate.shape[1]
    assert Bsz == 1
    J, PC = 32, 256
    T = NSEG * J
    hbm = pl.BlockSpec(memory_space=pl.ANY)
    vmem = pl.BlockSpec(memory_space=pltpu.VMEM)
    row = lambda v: v.reshape(1, -1)
    out = pl.pallas_call(
        functools.partial(_kernel, J=J, PC=PC),
        in_specs=[hbm, vmem, vmem, hbm, hbm, hbm, hbm, vmem, vmem, vmem, hbm, hbm, hbm],
        out_specs=hbm,
        out_shape=jax.ShapeDtypeStruct((NSEG, S // NSEG, D), F32),
        scratch_shapes=[
            pltpu.VMEM((NSEG, S // NSEG, D), BF16),
            pltpu.VMEM((P, D), BF16), pltpu.VMEM((P, D), BF16),
            pltpu.VMEM((D, P), BF16), pltpu.VMEM((D, P), BF16),
            pltpu.VMEM((D, F), BF16), pltpu.VMEM((D, F), BF16), pltpu.VMEM((F, D), BF16),
            pltpu.VMEM((D // 128, S, 128), F32),
            pltpu.VMEM((S, P), F32), pltpu.VMEM((S, P), F32),
            pltpu.VMEM((NSEG, P), F32), pltpu.VMEM((NSEG, P), F32),
            pltpu.VMEM((S, 128), F32),
            pltpu.VMEM((D // 128, T, 128), F32),
            pltpu.VMEM((2, NSEG, J, D), F32),
            pltpu.VMEM((2, T, P), BF16),
            pltpu.SemaphoreType.DMA((S // T,)),
            pltpu.SemaphoreType.DMA((2 * P // PC,)),
            pltpu.SemaphoreType.DMA((5,)),
            pltpu.SemaphoreType.DMA((2,)),
        ],
        compiler_params=pltpu.CompilerParams(vmem_limit_bytes=100 * 1024 * 1024),
    )(A_x.reshape(NSEG, S // NSEG, D), row(A_Lambda_re), row(A_Lambda_im), A_B_re, A_B_im,
      A_C_re, A_C_im, row(A_log_dt), row(A_Dskip), row(B_w_r), B_w_gate, B_w_up, B_w_down)
    return out.reshape(Bsz, S, D)
```

```python
import functools

import jax
import jax.numpy as jnp
import jax.experimental.pallas as pl
import jax.experimental.pallas.tpu as pltpu

F32 = jnp.float32
BF16 = jnp.bfloat16
NSEG = 8


def _rb(v):
    return v.astype(BF16).astype(F32)


def _layernorm_rows(x):
    d = x.shape[-1]
    m = jnp.sum(x, axis=-1, keepdims=True) * (1.0 / d)
    mb = _rb(m)
    xc = x - mb
    v = jnp.sum(xc * xc, axis=-1, keepdims=True) * (1.0 / d) - (m - mb) * (m - mb)
    s = _rb(jnp.sqrt(_rb(_rb(v) + 1e-5)))
    return _rb(_rb(xc) / s)


def _nt(a, b):
    return jax.lax.dot_general(a, b, (((1,), (1,)), ((), ())), preferred_element_type=F32)


def _nn(a, b):
    return jnp.dot(a, b, preferred_element_type=F32)


def _kernel(x_hbm, lre_ref, lim_ref, bre_hbm, bim_hbm, cre_hbm, cim_hbm, ldt_ref, dsk_ref,
            wr_ref, wg_hbm, wu_hbm, wd_hbm, o_hbm,
            xv, bre, bim, cre, cim, wg, wu, wd, res, bure, buim, hre, him, top, topi,
            car, stage, xb, hb, zero, xsel, yacc, sem_x, sem_b, sem_w, sem_o, *, J, PC):
    KD, S, _ = res.shape
    D = KD * 128
    P = bre.shape[0]
    F = wg.shape[1]
    SEG = S // NSEG
    NB = SEG // J
    T = NSEG * J
    NC = P // PC
    FC = F // (NB - 1)

    def x_copy(b):
        return pltpu.make_async_copy(
            x_hbm.at[:, pl.ds(b * J, J), :], xv.at[:, pl.ds(b * J, J), :], sem_x.at[b])

    def b_copy(c, src, dst, k):
        return pltpu.make_async_copy(
            src.at[pl.ds(c * PC, PC), :], dst.at[pl.ds(c * PC, PC), :], sem_b.at[2 * c + k])

    w_copies = [pltpu.make_async_copy(s_, d_, sem_w.at[i]) for i, (s_, d_) in enumerate(
        ((cre_hbm, cre), (cim_hbm, cim), (wg_hbm, wg), (wu_hbm, wu), (wd_hbm, wd)))]

    def o_copy(j0, n, k):
        return pltpu.make_async_copy(
            stage.at[:, pl.ds(j0, n), :], o_hbm.at[:, pl.ds(j0, n), :], sem_o.at[k])

    x_copy(0).start()
    for c in range(NC):
        b_copy(c, bre_hbm, bre, 0).start()
        b_copy(c, bim_hbm, bim, 1).start()
        if c == 0:
            x_copy(1).start()
    x_copy(2).start()

    row = lambda r: r[...].astype(F32).reshape(1, -1)
    lre, lim = row(lre_ref), row(lim_ref)
    dt = _rb(jnp.exp(row(ldt_ref)))
    mag = jnp.exp(dt * lre)
    are = mag * jnp.cos(dt * lim)
    aim = mag * jnp.sin(dt * lim)
    den = lre * lre + lim * lim
    kre8 = jnp.broadcast_to(2.0 * ((are - 1.0) * lre + aim * lim) / den, (NSEG, P))
    kim8 = jnp.broadcast_to(2.0 * (aim * lre - (are - 1.0) * lim) / den, (NSEG, P))
    are8 = jnp.broadcast_to(are, (NSEG, P))
    aim8 = jnp.broadcast_to(aim, (NSEG, P))
    dsk = 1.0 + row(dsk_ref)
    wr = row(wr_ref)

    hre[...] = jnp.zeros_like(hre)
    him[...] = jnp.zeros_like(him)
    yacc[...] = jnp.zeros_like(yacc)
    zero[...] = jnp.zeros_like(zero)

    JP = 16
    TP = JP * NSEG
    subd = jax.lax.broadcasted_iota(jnp.int32, (NSEG, 128), 0)
    top[0] = jnp.full((NSEG, 128), -jnp.inf, F32)
    top[1] = jnp.full((NSEG, 128), -jnp.inf, F32)
    topi[0] = subd * SEG
    topi[1] = subd * SEG + 1

    def permute(b, q):
        r0 = pl.multiple_of(b * T + q * TP, TP)
        j0 = pl.multiple_of(b * J + q * JP, JP)
        for s in range(NSEG):
            xs = xv[s, pl.ds(j0, JP), :].astype(F32)
            for k in range(KD):
                res[k, pl.ds(r0 + s, JP, stride=NSEG), :] = xs[:, k * 128:(k + 1) * 128]

    def norm(b, slot, g):
        rows = pl.ds(pl.multiple_of(b * T + g * 16, 16), 16)
        x = jnp.concatenate([res[k, rows, :] for k in range(KD)], axis=1)
        xn = _layernorm_rows(x)
        rs = x + xn * dsk
        for k in range(KD):
            res[k, rows, :] = rs[:, k * 128:(k + 1) * 128]
        xb[slot, g * 16:(g + 1) * 16, :] = xn.astype(BF16)
        r = jnp.broadcast_to(_rb(jnp.sum(xn * wr, axis=-1, keepdims=True)), (16, 128))
        b1, b2, i1, i2 = top[0], top[1], topi[0], topi[1]
        for j in range(2):
            rj = r[j * NSEG:(j + 1) * NSEG]
            tj = subd * SEG + (b * J + 2 * g + j)
            g1, g2 = rj > b1, rj > b2
            b2, i2 = jnp.where(g1, b1, jnp.where(g2, rj, b2)), jnp.where(g1, i1, jnp.where(g2, tj, i2))
            b1, i1 = jnp.where(g1, rj, b1), jnp.where(g1, tj, i1)
        top[0], top[1], topi[0], topi[1] = b1, b2, i1, i2

    def p1_block(b, slot, first=False, last=False):
        r0 = pl.multiple_of(b * T, T)
        NQ = J // JP
        NG = T // 16 // NC
        for c in range(NC):
            cs = slice(c * PC, (c + 1) * PC)
            if first:
                b_copy(c, bre_hbm, bre, 0).wait()
                b_copy(c, bim_hbm, bim, 1).wait()
            ure = _nt(xb[slot], bre[cs, :])
            uim = _nt(xb[slot], bim[cs, :])
            bure[pl.ds(r0, T), cs] = ure
            buim[pl.ds(r0, T), cs] = uim
            ar, ai = are8[:, cs], aim8[:, cs]
            hr, hi = hre[:, cs], him[:, cs]
            for j in range(J):
                js = slice(j * NSEG, (j + 1) * NSEG)
                hr, hi = (ar * hr + ure[js]) - ai * hi, (ar * hi + uim[js]) + ai * hr
            hre[:, cs] = hr
            him[:, cs] = hi
            if not last:
                if c % (NC // NQ) == 0:
                    permute(b + 1, c // (NC // NQ))
                for g in range(NG):
                    norm(b + 1, 1 - slot, c * NG + g)

    x_copy(0).wait()
    for q in range(J // JP):
        permute(0, q)
    for g in range(T // 16):
        norm(0, 0, g)
    x_copy(1).wait()
    with jax.named_scope('p1a'):
        p1_block(0, 0, first=True)
    for b in range(3, NB):
        x_copy(b).start()
    for cp in w_copies:
        cp.start()

    def p1_step(b, _):
        x_copy(b + 1).wait()
        p1_block(b, b % 2)

    with jax.named_scope('p1b'):
        jax.lax.fori_loop(1, NB - 1, p1_step, None)
    with jax.named_scope('p1c'):
        p1_block(NB - 1, (NB - 1) % 2, last=True)

    b1, b2, i1, i2 = top[0], top[1], topi[0], topi[1]
    m1 = jnp.max(b1)
    t1 = jnp.min(jnp.where(b1 == m1, i1, S))
    b1, i1 = jnp.where(i1 == t1, b2, b1), jnp.where(i1 == t1, i2, i1)
    m2 = jnp.max(b1)
    t2 = jnp.min(jnp.where(b1 == m2, i1, S))
    t1 = jnp.clip(t1, 0, S - 1)
    t2 = jnp.clip(t2, 0, S - 1)
    sub16 = jax.lax.broadcasted_iota(jnp.int32, (16, D), 0)

    def pick(t):
        s, j = t // SEG, t % SEG
        g = pl.multiple_of((j // 16) * 16, 16)
        xn = _layernorm_rows(xv[s, pl.ds(g, 16), :].astype(F32))
        return jnp.sum(jnp.where(sub16 == j % 16, xn, 0.0), axis=0, keepdims=True)

    xs = jnp.where(sub16 == 0, pick(t1), jnp.where(sub16 == 1, pick(t2), 0.0))
    xsel[:, :D // 2] = xs[:, :D // 2].astype(BF16)
    xsel[:, D // 2:] = (-xs[:, D // 2:]).astype(BF16)

    pr, pi = are8, aim8
    for _ in range(SEG.bit_length() - 1):
        pr, pi = pr * pr - pi * pi, 2.0 * pr * pi
    sub = jax.lax.broadcasted_iota(jnp.int32, (NSEG, P), 0)
    er, ei = hre[...], him[...]
    sh = 1
    while sh < NSEG:
        tr = jnp.where(sub >= sh, pltpu.roll(er, sh, 0), 0.0)
        ti = jnp.where(sub >= sh, pltpu.roll(ei, sh, 0), 0.0)
        er, ei = er + (pr * tr - pi * ti), ei + (pr * ti + pi * tr)
        pr, pi = pr * pr - pi * pi, 2.0 * pr * pi
        sh *= 2
    hre[...] = jnp.where(sub >= 1, pltpu.roll(er, 1, 0), 0.0)
    him[...] = jnp.where(sub >= 1, pltpu.roll(ei, 1, 0), 0.0)

    def scan(b, slot, c):
        r0 = pl.multiple_of(b * T, T)
        if True:
            cs = slice(c * 128, (c + 1) * 128)
            ar, ai, kr, ki = are8[:, cs], aim8[:, cs], kre8[:, cs], kim8[:, cs]
            hr, hi = hre[:, cs], him[:, cs]
            for j in range(0, J, 2):
                rows = pl.ds(pl.multiple_of(r0 + j * NSEG, 16), 16)
                ur, ui = bure[rows, cs], buim[rows, cs]
                hr0, hi0 = (ar * hr + ur[:8]) - ai * hi, (ar * hi + ui[:8]) + ai * hr
                hr, hi = (ar * hr0 + ur[8:]) - ai * hi0, (ar * hi0 + ui[8:]) + ai * hr0
                o = slice(j * NSEG, (j + 2) * NSEG)
                hb[slot, 0, c, o, :] = jnp.concatenate([kr * hr0 - ki * hi0, kr * hr - ki * hi], 0).astype(BF16)
                hb[slot, 1, c, o, :] = jnp.concatenate([kr * hi0 + ki * hr0, kr * hi + ki * hr], 0).astype(BF16)
            hre[:, cs] = hr
            him[:, cs] = hi

    def ffn_pieces(b):
        f0 = pl.multiple_of(b * FC, FC)
        acts = []
        for n in range(FC // 128):
            fs = pl.ds(pl.multiple_of(f0 + n * 128, 128), 128)
            gu = []
            for w in (wg, wu):
                a = _nn(xsel[:, :D // 2], w[:D // 2, fs])
                yield
                gu.append(_rb(a - _nn(xsel[:, D // 2:], w[D // 2:, fs])))
                yield
            g, u = gu
            acts.append((_rb(g * jax.nn.sigmoid(g)) * u).astype(BF16))
        act = jnp.concatenate(acts, axis=1)
        yield
        yield
        for k in range(KD):
            ks = slice(k * 128, (k + 1) * 128)
            yacc[:, ks] += _nn(act, wd[pl.ds(f0, FC), ks])[:8]
            yield

    def hcat(slot, part, half):
        n = P // 256
        return jnp.concatenate([hb[slot, part, half * n + c] for c in range(n)], axis=1)

    def p2_block(b, slot, last=False):
        r0 = pl.multiple_of(b * T, T)
        ffn = iter(()) if last else ffn_pieces(b)
        H = P // 2
        for k in range(KD):
            ks = slice(k * 128, (k + 1) * 128)
            y = res[k, pl.ds(r0, T), :]
            y = y + _nt(hcat(slot, 0, 0), cre[ks, :H])
            next(ffn, None)
            y = y - _nt(hcat(slot, 1, 0), cim[ks, :H])
            next(ffn, None)
            y = y + _nt(hcat(slot, 0, 1), cre[ks, H:])
            next(ffn, None)
            y = y - _nt(hcat(slot, 1, 1), cim[ks, H:])
            next(ffn, None)
            if not last:
                scan(b + 1, 1 - slot, k)
            car[k] = y
            for s in range(NSEG):
                stage[s, pl.ds(pl.multiple_of(b * J, J), J), ks] = car[k, pl.ds(s, J, stride=NSEG), :]
        if not last:
            o_copy(pl.multiple_of(b * J, J), J, 0).start()

    for c in range(P // 128):
        scan(0, 0, c)
    for cp in w_copies:
        cp.wait()
    with jax.named_scope('p2'):
        jax.lax.fori_loop(0, NB - 1, lambda b, _: p2_block(b, b % 2), None)
    with jax.named_scope('p2l'):
        p2_block(NB - 1, (NB - 1) % 2, last=True)

    o_copy(0, (NB - 1) * J, 0).wait()
    for k, (t, m) in enumerate(((t1, m1), (t2, m2))):
        gate = jax.nn.sigmoid(jnp.full((1, D), m, F32))
        srow = pl.ds(t % SEG, 1)
        stage[t // SEG, srow, :] = stage[t // SEG, srow, :] + yacc[k:k + 1, :] * gate
    o_copy((NB - 1) * J, J, 0).start()
    g1 = pl.multiple_of((t1 % SEG) // 8 * 8, 8)
    g2 = pl.multiple_of((t2 % SEG) // 8 * 8, 8)
    redo1 = g1 < (NB - 1) * J
    redo2 = jnp.logical_and(g2 < (NB - 1) * J, g2 != g1)
    pl.when(redo1)(lambda: o_copy(g1, 8, 1).start())
    pl.when(redo2)(lambda: o_copy(g2, 8, 2).start())
    pl.when(redo1)(lambda: o_copy(g1, 8, 1).wait())
    pl.when(redo2)(lambda: o_copy(g2, 8, 2).wait())
    o_copy((NB - 1) * J, J, 0).wait()


@jax.jit
def pallas_parallel_sum__ssm_conv_s5__moe_arch_mod__prompt_kernel(
    A_x: jax.Array,
    A_Lambda_re: jax.Array,
    A_Lambda_im: jax.Array,
    A_B_re: jax.Array,
    A_B_im: jax.Array,
    A_C_re: jax.Array,
    A_C_im: jax.Array,
    A_log_dt: jax.Array,
    A_Dskip: jax.Array,
    B_x: jax.Array,
    B_w_r: jax.Array,
    B_w_gate: jax.Array,
    B_w_up: jax.Array,
    B_w_down: jax.Array,
):
    del B_x
    Bsz, S, D = A_x.shape
    P = A_B_re.shape[0]
    F = B_w_gate.shape[1]
    assert Bsz == 1
    J, PC = 32, 256
    T = NSEG * J
    hbm = pl.BlockSpec(memory_space=pl.ANY)
    vmem = pl.BlockSpec(memory_space=pltpu.VMEM)
    out = pl.pallas_call(
        functools.partial(_kernel, J=J, PC=PC),
        in_specs=[hbm, vmem, vmem, hbm, hbm, hbm, hbm, vmem, vmem, vmem, hbm, hbm, hbm],
        out_specs=hbm,
        out_shape=jax.ShapeDtypeStruct((NSEG, S // NSEG, D), F32),
        scratch_shapes=[
            pltpu.VMEM((NSEG, S // NSEG, D), BF16),
            pltpu.VMEM((P, D), BF16), pltpu.VMEM((P, D), BF16),
            pltpu.VMEM((D, P), BF16), pltpu.VMEM((D, P), BF16),
            pltpu.VMEM((D, F), BF16), pltpu.VMEM((D, F), BF16), pltpu.VMEM((F, D), BF16),
            pltpu.VMEM((D // 128, S, 128), F32),
            pltpu.VMEM((S, P), F32), pltpu.VMEM((S, P), F32),
            pltpu.VMEM((NSEG, P), F32), pltpu.VMEM((NSEG, P), F32),
            pltpu.VMEM((2, NSEG, 128), F32), pltpu.VMEM((2, NSEG, 128), jnp.int32),
            pltpu.VMEM((D // 128, T, 128), F32),
            pltpu.VMEM((NSEG, S // NSEG, D), F32),
            pltpu.VMEM((2, T, D), BF16),
            pltpu.VMEM((2, 2, P // 128, T, 128), BF16),
            pltpu.VMEM((8, 128), jnp.int32),
            pltpu.VMEM((16, D), BF16), pltpu.VMEM((8, D), F32),
            pltpu.SemaphoreType.DMA((S // T,)),
            pltpu.SemaphoreType.DMA((2 * P // PC,)),
            pltpu.SemaphoreType.DMA((5,)),
            pltpu.SemaphoreType.DMA((3,)),
        ],
        compiler_params=pltpu.CompilerParams(vmem_limit_bytes=100 * 1024 * 1024),
    )(A_x.reshape(NSEG, S // NSEG, D), A_Lambda_re, A_Lambda_im, A_B_re, A_B_im,
      A_C_re, A_C_im, A_log_dt, A_Dskip, B_w_r, B_w_gate, B_w_up, B_w_down)
    return out.reshape(Bsz, S, D)
```

```python
import functools

import jax
import jax.numpy as jnp
import jax.experimental.pallas as pl
import jax.experimental.pallas.tpu as pltpu

F32 = jnp.float32
BF16 = jnp.bfloat16
NSEG = 8


def _rb(v):
    return v.astype(BF16).astype(F32)


def _layernorm_rows(x):
    d = x.shape[-1]
    m = jnp.sum(x, axis=-1, keepdims=True) * (1.0 / d)
    mb = _rb(m)
    xc = x - mb
    v = jnp.sum(xc * xc, axis=-1, keepdims=True) * (1.0 / d) - (m - mb) * (m - mb)
    s = _rb(jnp.sqrt(_rb(_rb(v) + 1e-5)))
    return _rb(_rb(xc) / s)


def _nt(a, b):
    return jax.lax.dot_general(a, b, (((1,), (1,)), ((), ())), preferred_element_type=F32)


def _nn(a, b):
    return jnp.dot(a, b, preferred_element_type=F32)


def _kernel(x_hbm, lre_ref, lim_ref, bre_hbm, bim_hbm, cre_hbm, cim_hbm, ldt_ref, dsk_ref,
            wr_ref, wg_hbm, wu_hbm, wd_hbm, o_hbm,
            xv, bre, bim, cre, cim, wg, wu, wd, res, bure, buim, hre, him, top, topi,
            car, stage, xb, hb, zero, xsel, yacc, sem_x, sem_b, sem_w, sem_o, *, J, PC):
    KD, S, _ = res.shape
    D = KD * 128
    P = bre.shape[0]
    F = wg.shape[1]
    SEG = S // NSEG
    NB = SEG // J
    T = NSEG * J
    NC = P // PC
    FC = F // (NB - 1)

    def x_copy(b):
        return pltpu.make_async_copy(
            x_hbm.at[:, pl.ds(b * J, J), :], xv.at[:, pl.ds(b * J, J), :], sem_x.at[b])

    def b_copy(c, src, dst, k):
        return pltpu.make_async_copy(
            src.at[pl.ds(c * PC, PC), :], dst.at[pl.ds(c * PC, PC), :], sem_b.at[2 * c + k])

    w_copies = [pltpu.make_async_copy(s_, d_, sem_w.at[i]) for i, (s_, d_) in enumerate(
        ((cre_hbm, cre), (cim_hbm, cim), (wg_hbm, wg), (wu_hbm, wu), (wd_hbm, wd)))]

    def o_copy(j0, n, k):
        return pltpu.make_async_copy(
            stage.at[:, pl.ds(j0, n), :], o_hbm.at[:, pl.ds(j0, n), :], sem_o.at[k])

    x_copy(0).start()
    x_copy(1).start()
    b_copy(0, bre_hbm, bre, 0).start()
    b_copy(0, bim_hbm, bim, 1).start()

    row = lambda r: r[...].astype(F32).reshape(1, -1)
    lre, lim = row(lre_ref), row(lim_ref)
    dt = _rb(jnp.exp(row(ldt_ref)))
    mag = jnp.exp(dt * lre)
    are = mag * jnp.cos(dt * lim)
    aim = mag * jnp.sin(dt * lim)
    den = lre * lre + lim * lim
    kre8 = jnp.broadcast_to(2.0 * ((are - 1.0) * lre + aim * lim) / den, (NSEG, P))
    kim8 = jnp.broadcast_to(2.0 * (aim * lre - (are - 1.0) * lim) / den, (NSEG, P))
    are8 = jnp.broadcast_to(are, (NSEG, P))
    aim8 = jnp.broadcast_to(aim, (NSEG, P))
    dsk = 1.0 + row(dsk_ref)
    wr = row(wr_ref)

    hre[...] = jnp.zeros_like(hre)
    him[...] = jnp.zeros_like(him)
    yacc[...] = jnp.zeros_like(yacc)
    zero[...] = jnp.zeros_like(zero)

    JP = 16
    TP = JP * NSEG
    subd = jax.lax.broadcasted_iota(jnp.int32, (NSEG, 128), 0)
    top[0] = jnp.full((NSEG, 128), -jnp.inf, F32)
    top[1] = jnp.full((NSEG, 128), -jnp.inf, F32)
    topi[0] = subd * SEG
    topi[1] = subd * SEG + 1

    def permute(b, q):
        r0 = pl.multiple_of(b * T + q * TP, TP)
        j0 = pl.multiple_of(b * J + q * JP, JP)
        for s in range(NSEG):
            xs = xv[s, pl.ds(j0, JP), :].astype(F32)
            for k in range(KD):
                res[k, pl.ds(r0 + s, JP, stride=NSEG), :] = xs[:, k * 128:(k + 1) * 128]

    def norm(b, slot, g):
        rows = pl.ds(pl.multiple_of(b * T + g * 16, 16), 16)
        x = jnp.concatenate([res[k, rows, :] for k in range(KD)], axis=1)
        xn = _layernorm_rows(x)
        rs = x + xn * dsk
        for k in range(KD):
            res[k, rows, :] = rs[:, k * 128:(k + 1) * 128]
        xb[slot, g * 16:(g + 1) * 16, :] = xn.astype(BF16)
        r = jnp.broadcast_to(_rb(jnp.sum(xn * wr, axis=-1, keepdims=True)), (16, 128))
        b1, b2, i1, i2 = top[0], top[1], topi[0], topi[1]
        for j in range(2):
            rj = r[j * NSEG:(j + 1) * NSEG]
            tj = subd * SEG + (b * J + 2 * g + j)
            g1, g2 = rj > b1, rj > b2
            b2, i2 = jnp.where(g1, b1, jnp.where(g2, rj, b2)), jnp.where(g1, i1, jnp.where(g2, tj, i2))
            b1, i1 = jnp.where(g1, rj, b1), jnp.where(g1, tj, i1)
        top[0], top[1], topi[0], topi[1] = b1, b2, i1, i2

    def p1_block(b, slot, first=False, last=False):
        r0 = pl.multiple_of(b * T, T)
        NT = P // 128
        for c in range(NT):
            cs = slice(c * 128, (c + 1) * 128)
            if first and c % (NT // NC) == 0:
                cc = c // (NT // NC)
                b_copy(cc, bre_hbm, bre, 0).wait()
                b_copy(cc, bim_hbm, bim, 1).wait()
                if cc + 2 < NC:
                    b_copy(cc + 2, bre_hbm, bre, 0).start()
                    b_copy(cc + 2, bim_hbm, bim, 1).start()
                elif cc + 2 == NC:
                    x_copy(2).start()
            us = []
            for part, (w, bu) in enumerate(((bre, bure), (bim, buim))):
                u = _nt(xb[slot], w[cs, :])
                bu[pl.ds(r0, T), cs] = u
                us.append(u)
                if not last:
                    g = 2 * c + part
                    if g % (TP // 16) == 0:
                        permute(b + 1, g // (TP // 16))
                    norm(b + 1, 1 - slot, g)
                else:
                    xb[1 - slot, :16, :256] = jnp.zeros((16, 256), BF16)
            ure, uim = us
            ar, ai = are8[:, cs], aim8[:, cs]
            hr, hi = hre[:, cs], him[:, cs]
            for j in range(J):
                js = slice(j * NSEG, (j + 1) * NSEG)
                hr, hi = (ar * hr + ure[js]) - ai * hi, (ar * hi + uim[js]) + ai * hr
            hre[:, cs] = hr
            him[:, cs] = hi

    x_copy(0).wait()
    b_copy(1, bre_hbm, bre, 0).start()
    b_copy(1, bim_hbm, bim, 1).start()
    for q in range(J // JP):
        permute(0, q)
    for g in range(T // 16):
        norm(0, 0, g)
    x_copy(1).wait()
    p1_block(0, 0, first=True)
    for b in range(3, NB):
        x_copy(b).start()
    for cp in w_copies:
        cp.start()

    def p1_step(b, _):
        x_copy(b + 1).wait()
        p1_block(b, b % 2)

    jax.lax.fori_loop(1, NB - 1, p1_step, None)
    b1, b2, i1, i2 = top[0], top[1], topi[0], topi[1]
    m1 = jnp.max(b1)
    t1 = jnp.min(jnp.where(b1 == m1, i1, S))
    b1, i1 = jnp.where(i1 == t1, b2, b1), jnp.where(i1 == t1, i2, i1)
    m2 = jnp.max(b1)
    t2 = jnp.min(jnp.where(b1 == m2, i1, S))
    t1 = jnp.clip(t1, 0, S - 1)
    t2 = jnp.clip(t2, 0, S - 1)
    sub16 = jax.lax.broadcasted_iota(jnp.int32, (16, D), 0)

    def pick(t):
        s, j = t // SEG, t % SEG
        g = pl.multiple_of((j // 16) * 16, 16)
        xn = _layernorm_rows(xv[s, pl.ds(g, 16), :].astype(F32))
        return jnp.sum(jnp.where(sub16 == j % 16, xn, 0.0), axis=0, keepdims=True)

    xs = jnp.where(sub16 == 0, pick(t1), jnp.where(sub16 == 1, pick(t2), 0.0))
    xsel[:, :D // 2] = xs[:, :D // 2].astype(BF16)
    xsel[:, D // 2:] = (-xs[:, D // 2:]).astype(BF16)

    p1_block(NB - 1, (NB - 1) % 2, last=True)

    pr, pi = are8, aim8
    for _ in range(SEG.bit_length() - 1):
        pr, pi = pr * pr - pi * pi, 2.0 * pr * pi
    sub = jax.lax.broadcasted_iota(jnp.int32, (NSEG, P), 0)
    er, ei = hre[...], him[...]
    sh = 1
    while sh < NSEG:
        tr = jnp.where(sub >= sh, pltpu.roll(er, sh, 0), 0.0)
        ti = jnp.where(sub >= sh, pltpu.roll(ei, sh, 0), 0.0)
        er, ei = er + (pr * tr - pi * ti), ei + (pr * ti + pi * tr)
        pr, pi = pr * pr - pi * pi, 2.0 * pr * pi
        sh *= 2
    hre[...] = jnp.where(sub >= 1, pltpu.roll(er, 1, 0), 0.0)
    him[...] = jnp.where(sub >= 1, pltpu.roll(ei, 1, 0), 0.0)

    def scan(b, slot, c):
        r0 = pl.multiple_of(b * T, T)
        if True:
            cs = slice(c * 128, (c + 1) * 128)
            ar, ai, kr, ki = are8[:, cs], aim8[:, cs], kre8[:, cs], kim8[:, cs]
            hr, hi = hre[:, cs], him[:, cs]
            for j in range(0, J, 2):
                rows = pl.ds(pl.multiple_of(r0 + j * NSEG, 16), 16)
                ur, ui = bure[rows, cs], buim[rows, cs]
                hr0, hi0 = (ar * hr + ur[:8]) - ai * hi, (ar * hi + ui[:8]) + ai * hr
                hr, hi = (ar * hr0 + ur[8:]) - ai * hi0, (ar * hi0 + ui[8:]) + ai * hr0
                o = slice(j * NSEG, (j + 2) * NSEG)
                hb[slot, 0, c, o, :] = jnp.concatenate([kr * hr0 - ki * hi0, kr * hr - ki * hi], 0).astype(BF16)
                hb[slot, 1, c, o, :] = jnp.concatenate([kr * hi0 + ki * hr0, kr * hi + ki * hr], 0).astype(BF16)
            hre[:, cs] = hr
            him[:, cs] = hi

    def ffn_pieces(b):
        f0 = pl.multiple_of(b * FC, FC)
        acts = []
        for n in range(FC // 128):
            fs = pl.ds(pl.multiple_of(f0 + n * 128, 128), 128)
            gu = []
            for w in (wg, wu):
                a = _nn(xsel[:, :D // 2], w[:D // 2, fs])
                yield
                gu.append(_rb(a - _nn(xsel[:, D // 2:], w[D // 2:, fs])))
                yield
            g, u = gu
            acts.append((_rb(g * jax.nn.sigmoid(g)) * u).astype(BF16))
        act = jnp.concatenate(acts, axis=1)
        yield
        yield
        for k in range(KD):
            ks = slice(k * 128, (k + 1) * 128)
            yacc[:, ks] += _nn(act, wd[pl.ds(f0, FC), ks])[:8]
            yield

    def hcat(slot, part, half):
        n = P // 256
        return jnp.concatenate([hb[slot, part, half * n + c] for c in range(n)], axis=1)

    def p2_block(b, slot, last=False):
        r0 = pl.multiple_of(b * T, T)
        ffn = iter(()) if last else ffn_pieces(b)
        H = P // 2
        for k in range(KD):
            ks = slice(k * 128, (k + 1) * 128)
            y = res[k, pl.ds(r0, T), :]
            y = y + _nt(hcat(slot, 0, 0), cre[ks, :H])
            next(ffn, None)
            y = y - _nt(hcat(slot, 1, 0), cim[ks, :H])
            next(ffn, None)
            y = y + _nt(hcat(slot, 0, 1), cre[ks, H:])
            next(ffn, None)
            y = y - _nt(hcat(slot, 1, 1), cim[ks, H:])
            next(ffn, None)
            if not last:
                scan(b + 1, 1 - slot, k)
            car[k] = y
            for s in range(NSEG):
                stage[s, pl.ds(pl.multiple_of(b * J, J), J), ks] = car[k, pl.ds(s, J, stride=NSEG), :]
            if last and k in (5, 7):
                cols = pl.ds(0, 768) if k == 5 else pl.ds(768, 256)
                pltpu.make_async_copy(stage.at[:, pl.ds(b * J, J), cols],
                                      o_hbm.at[:, pl.ds(b * J, J), cols], sem_o.at[3]).start()
        if not last:
            o_copy(pl.multiple_of(b * J, J), J, 0).start()

    for c in range(P // 128):
        scan(0, 0, c)
    for cp in w_copies:
        cp.wait()
    jax.lax.fori_loop(0, NB - 1, lambda b, _: p2_block(b, b % 2), None)

    routed = [(t // SEG, t % SEG, yacc[k:k + 1, :] * jax.nn.sigmoid(jnp.full((1, D), m, F32)))
              for k, (t, m) in enumerate(((t1, m1), (t2, m2)))]
    JL = (NB - 1) * J
    for s, j, yk in routed:
        @pl.when(j >= JL)
        def _():
            prow = pl.ds(j * NSEG + s, 1)
            for q in range(KD):
                res[q, prow, :] = res[q, prow, :] + yk[:, q * 128:(q + 1) * 128]

    p2_block(NB - 1, (NB - 1) % 2, last=True)

    o_copy(0, JL, 0).wait()
    for s, j, yk in routed:
        @pl.when(j < JL)
        def _():
            srow = pl.ds(jnp.minimum(j, SEG - 1), 1)
            stage[s, srow, :] = stage[s, srow, :] + yk
    g1 = pl.multiple_of(routed[0][1] // 8 * 8, 8)
    g2 = pl.multiple_of(routed[1][1] // 8 * 8, 8)
    redo1 = g1 < JL
    redo2 = jnp.logical_and(g2 < JL, g2 != g1)
    pl.when(redo1)(lambda: o_copy(g1, 8, 1).start())
    pl.when(redo2)(lambda: o_copy(g2, 8, 2).start())
    pl.when(redo1)(lambda: o_copy(g1, 8, 1).wait())
    pl.when(redo2)(lambda: o_copy(g2, 8, 2).wait())
    o_copy(JL, J, 3).wait()


@jax.jit
def pallas_parallel_sum__ssm_conv_s5__moe_arch_mod__prompt_kernel(
    A_x: jax.Array,
    A_Lambda_re: jax.Array,
    A_Lambda_im: jax.Array,
    A_B_re: jax.Array,
    A_B_im: jax.Array,
    A_C_re: jax.Array,
    A_C_im: jax.Array,
    A_log_dt: jax.Array,
    A_Dskip: jax.Array,
    B_x: jax.Array,
    B_w_r: jax.Array,
    B_w_gate: jax.Array,
    B_w_up: jax.Array,
    B_w_down: jax.Array,
):
    del B_x
    Bsz, S, D = A_x.shape
    P = A_B_re.shape[0]
    F = B_w_gate.shape[1]
    assert Bsz == 1
    J, PC = 32, 256
    T = NSEG * J
    hbm = pl.BlockSpec(memory_space=pl.ANY)
    vmem = pl.BlockSpec(memory_space=pltpu.VMEM)
    out = pl.pallas_call(
        functools.partial(_kernel, J=J, PC=PC),
        in_specs=[hbm, vmem, vmem, hbm, hbm, hbm, hbm, vmem, vmem, vmem, hbm, hbm, hbm],
        out_specs=hbm,
        out_shape=jax.ShapeDtypeStruct((NSEG, S // NSEG, D), F32),
        scratch_shapes=[
            pltpu.VMEM((NSEG, S // NSEG, D), BF16),
            pltpu.VMEM((P, D), BF16), pltpu.VMEM((P, D), BF16),
            pltpu.VMEM((D, P), BF16), pltpu.VMEM((D, P), BF16),
            pltpu.VMEM((D, F), BF16), pltpu.VMEM((D, F), BF16), pltpu.VMEM((F, D), BF16),
            pltpu.VMEM((D // 128, S, 128), F32),
            pltpu.VMEM((S, P), F32), pltpu.VMEM((S, P), F32),
            pltpu.VMEM((NSEG, P), F32), pltpu.VMEM((NSEG, P), F32),
            pltpu.VMEM((2, NSEG, 128), F32), pltpu.VMEM((2, NSEG, 128), jnp.int32),
            pltpu.VMEM((D // 128, T, 128), F32),
            pltpu.VMEM((NSEG, S // NSEG, D), F32),
            pltpu.VMEM((2, T, D), BF16),
            pltpu.VMEM((2, 2, P // 128, T, 128), BF16),
            pltpu.VMEM((8, 128), jnp.int32),
            pltpu.VMEM((16, D), BF16), pltpu.VMEM((8, D), F32),
            pltpu.SemaphoreType.DMA((S // T,)),
            pltpu.SemaphoreType.DMA((2 * P // PC,)),
            pltpu.SemaphoreType.DMA((5,)),
            pltpu.SemaphoreType.DMA((4,)),
        ],
        compiler_params=pltpu.CompilerParams(vmem_limit_bytes=100 * 1024 * 1024),
    )(A_x.reshape(NSEG, S // NSEG, D), A_Lambda_re, A_Lambda_im, A_B_re, A_B_im,
      A_C_re, A_C_im, A_log_dt, A_Dskip, B_w_r, B_w_gate, B_w_up, B_w_down)
    return out.reshape(Bsz, S, D)
```

```python
import functools

import jax
import jax.numpy as jnp
import jax.experimental.pallas as pl
import jax.experimental.pallas.tpu as pltpu

F32 = jnp.float32
BF16 = jnp.bfloat16
NSEG = 8


def _rb(v):
    return v.astype(BF16).astype(F32)


def _layernorm_rows(x):
    d = x.shape[-1]
    m = jnp.sum(x, axis=-1, keepdims=True) * (1.0 / d)
    mb = _rb(m)
    xc = x - mb
    v = jnp.sum(xc * xc, axis=-1, keepdims=True) * (1.0 / d) - (m - mb) * (m - mb)
    s = _rb(jnp.sqrt(_rb(_rb(v) + 1e-5)))
    return _rb(_rb(xc) / s)


def _nt(a, b):
    return jax.lax.dot_general(a, b, (((1,), (1,)), ((), ())), preferred_element_type=F32)


def _nn(a, b):
    return jnp.dot(a, b, preferred_element_type=F32)


def _kernel(x_hbm, lre_ref, lim_ref, bre_hbm, bim_hbm, cre_hbm, cim_hbm, ldt_ref, dsk_ref,
            wr_ref, wg_hbm, wu_hbm, wd_hbm, o_hbm,
            xv, bre, bim, cre, cim, wg, wu, wd, res, bure, buim, hre, him, top, topi,
            car, stage, xb, hb, xnf, xsel, yacc, sem_x, sem_b, sem_w, sem_o, *, J, PC):
    KD, S, _ = res.shape
    D = KD * 128
    P = bre.shape[0]
    F = wg.shape[1]
    SEG = S // NSEG
    NB = SEG // J
    T = NSEG * J
    NC = P // PC
    FC = F // (NB - 1)

    def x_copy(b):
        return pltpu.make_async_copy(
            x_hbm.at[:, pl.ds(b * J, J), :], xv.at[:, pl.ds(b * J, J), :], sem_x.at[b])

    def b_copy(c, src, dst, k):
        return pltpu.make_async_copy(
            src.at[pl.ds(c * PC, PC), :], dst.at[pl.ds(c * PC, PC), :], sem_b.at[2 * c + k])

    w_copies = [pltpu.make_async_copy(s_, d_, sem_w.at[i]) for i, (s_, d_) in enumerate(
        ((cre_hbm, cre), (cim_hbm, cim), (wg_hbm, wg), (wu_hbm, wu), (wd_hbm, wd)))]

    def o_copy(j0, n, k):
        return pltpu.make_async_copy(
            stage.at[:, pl.ds(j0, n), :], o_hbm.at[:, pl.ds(j0, n), :], sem_o.at[k])

    x_copy(0).start()
    x_copy(1).start()
    b_copy(0, bre_hbm, bre, 0).start()
    b_copy(0, bim_hbm, bim, 1).start()

    row = lambda r: r[...].astype(F32).reshape(1, -1)
    lre, lim = row(lre_ref), row(lim_ref)
    dt = _rb(jnp.exp(row(ldt_ref)))
    mag = jnp.exp(dt * lre)
    are = mag * jnp.cos(dt * lim)
    aim = mag * jnp.sin(dt * lim)
    den = lre * lre + lim * lim
    kre8 = jnp.broadcast_to(2.0 * ((are - 1.0) * lre + aim * lim) / den, (NSEG, P))
    kim8 = jnp.broadcast_to(2.0 * (aim * lre - (are - 1.0) * lim) / den, (NSEG, P))
    are8 = jnp.broadcast_to(are, (NSEG, P))
    aim8 = jnp.broadcast_to(aim, (NSEG, P))
    dsk = 1.0 + row(dsk_ref)
    wr = row(wr_ref)

    hre[...] = jnp.zeros_like(hre)
    him[...] = jnp.zeros_like(him)
    yacc[...] = jnp.zeros_like(yacc)

    JP = 16
    TP = JP * NSEG
    subd = jax.lax.broadcasted_iota(jnp.int32, (NSEG, 128), 0)
    top[0] = jnp.full((NSEG, 128), -jnp.inf, F32)
    top[1] = jnp.full((NSEG, 128), -jnp.inf, F32)
    topi[0] = subd * SEG
    topi[1] = subd * SEG + 1

    def permute(b, q):
        r0 = pl.multiple_of(b * T + q * TP, TP)
        j0 = pl.multiple_of(b * J + q * JP, JP)
        for s in range(NSEG):
            xs = xv[s, pl.ds(j0, JP), :].astype(F32)
            for k in range(KD):
                res[k, pl.ds(r0 + s, JP, stride=NSEG), :] = xs[:, k * 128:(k + 1) * 128]

    def norm(b, slot, g):
        rows = pl.ds(pl.multiple_of(b * T + g * 16, 16), 16)
        x = jnp.concatenate([res[k, rows, :] for k in range(KD)], axis=1)
        xn = _layernorm_rows(x)
        xb[slot, g * 16:(g + 1) * 16, :] = xn.astype(BF16)
        xnf[rows, :] = xn.astype(BF16)
        r = jnp.broadcast_to(_rb(jnp.sum(xn * wr, axis=-1, keepdims=True)), (16, 128))
        b1, b2, i1, i2 = top[0], top[1], topi[0], topi[1]
        for j in range(2):
            rj = r[j * NSEG:(j + 1) * NSEG]
            tj = subd * SEG + (b * J + 2 * g + j)
            g1, g2 = rj > b1, rj > b2
            b2, i2 = jnp.where(g1, b1, jnp.where(g2, rj, b2)), jnp.where(g1, i1, jnp.where(g2, tj, i2))
            b1, i1 = jnp.where(g1, rj, b1), jnp.where(g1, tj, i1)
        top[0], top[1], topi[0], topi[1] = b1, b2, i1, i2

    def p1_block(b, slot, first=False, last=False):
        r0 = pl.multiple_of(b * T, T)
        NT = P // 128
        for c in range(NT):
            cs = slice(c * 128, (c + 1) * 128)
            if first and c % (NT // NC) == 0:
                cc = c // (NT // NC)
                b_copy(cc, bre_hbm, bre, 0).wait()
                b_copy(cc, bim_hbm, bim, 1).wait()
                if cc + 2 < NC:
                    b_copy(cc + 2, bre_hbm, bre, 0).start()
                    b_copy(cc + 2, bim_hbm, bim, 1).start()
                elif cc + 2 == NC:
                    x_copy(2).start()
            us = []
            for part, (w, bu) in enumerate(((bre, bure), (bim, buim))):
                u = _nt(xb[slot], w[cs, :])
                bu[pl.ds(r0, T), cs] = u
                us.append(u)
                if not last:
                    g = 2 * c + part
                    if g == 0:
                        permute(b + 1, 0)
                        permute(b + 1, 1)
                    norm(b + 1, 1 - slot, g)
                else:
                    xb[1 - slot, :16, :256] = jnp.zeros((16, 256), BF16)
            ure, uim = us
            ar, ai = are8[:, cs], aim8[:, cs]
            hr, hi = hre[:, cs], him[:, cs]
            for j in range(J):
                js = slice(j * NSEG, (j + 1) * NSEG)
                hr, hi = (ar * hr + ure[js]) - ai * hi, (ar * hi + uim[js]) + ai * hr
            hre[:, cs] = hr
            him[:, cs] = hi

    x_copy(0).wait()
    b_copy(1, bre_hbm, bre, 0).start()
    b_copy(1, bim_hbm, bim, 1).start()
    for q in range(J // JP):
        permute(0, q)
    for g in range(T // 16):
        norm(0, 0, g)
    x_copy(1).wait()
    p1_block(0, 0, first=True)
    for b in range(3, NB):
        x_copy(b).start()
    for cp in w_copies:
        cp.start()

    def p1_step(b, _):
        x_copy(b + 1).wait()
        p1_block(b, b % 2)

    jax.lax.fori_loop(1, NB - 1, p1_step, None)
    b1, b2, i1, i2 = top[0], top[1], topi[0], topi[1]
    m1 = jnp.max(b1)
    t1 = jnp.min(jnp.where(b1 == m1, i1, S))
    b1, i1 = jnp.where(i1 == t1, b2, b1), jnp.where(i1 == t1, i2, i1)
    m2 = jnp.max(b1)
    t2 = jnp.min(jnp.where(b1 == m2, i1, S))
    t1 = jnp.clip(t1, 0, S - 1)
    t2 = jnp.clip(t2, 0, S - 1)
    sub16 = jax.lax.broadcasted_iota(jnp.int32, (16, D), 0)

    def pick(t):
        s, j = t // SEG, t % SEG
        g = pl.multiple_of((j // 16) * 16, 16)
        xn = _layernorm_rows(xv[s, pl.ds(g, 16), :].astype(F32))
        return jnp.sum(jnp.where(sub16 == j % 16, xn, 0.0), axis=0, keepdims=True)

    xs = jnp.where(sub16 == 0, pick(t1), jnp.where(sub16 == 1, pick(t2), 0.0))
    xsel[:, :D // 2] = xs[:, :D // 2].astype(BF16)
    xsel[:, D // 2:] = (-xs[:, D // 2:]).astype(BF16)

    p1_block(NB - 1, (NB - 1) % 2, last=True)

    pr, pi = are8, aim8
    for _ in range(SEG.bit_length() - 1):
        pr, pi = pr * pr - pi * pi, 2.0 * pr * pi
    sub = jax.lax.broadcasted_iota(jnp.int32, (NSEG, P), 0)
    er, ei = hre[...], him[...]
    sh = 1
    while sh < NSEG:
        tr = jnp.where(sub >= sh, pltpu.roll(er, sh, 0), 0.0)
        ti = jnp.where(sub >= sh, pltpu.roll(ei, sh, 0), 0.0)
        er, ei = er + (pr * tr - pi * ti), ei + (pr * ti + pi * tr)
        pr, pi = pr * pr - pi * pi, 2.0 * pr * pi
        sh *= 2
    hre[...] = jnp.where(sub >= 1, pltpu.roll(er, 1, 0), 0.0)
    him[...] = jnp.where(sub >= 1, pltpu.roll(ei, 1, 0), 0.0)

    def scan(b, slot, c):
        r0 = pl.multiple_of(b * T, T)
        if True:
            cs = slice(c * 128, (c + 1) * 128)
            ar, ai, kr, ki = are8[:, cs], aim8[:, cs], kre8[:, cs], kim8[:, cs]
            hr, hi = hre[:, cs], him[:, cs]
            for j in range(0, J, 2):
                rows = pl.ds(pl.multiple_of(r0 + j * NSEG, 16), 16)
                ur, ui = bure[rows, cs], buim[rows, cs]
                hr0, hi0 = (ar * hr + ur[:8]) - ai * hi, (ar * hi + ui[:8]) + ai * hr
                hr, hi = (ar * hr0 + ur[8:]) - ai * hi0, (ar * hi0 + ui[8:]) + ai * hr0
                o = slice(j * NSEG, (j + 2) * NSEG)
                hb[slot, 0, c, o, :] = jnp.concatenate([kr * hr0 - ki * hi0, kr * hr - ki * hi], 0).astype(BF16)
                hb[slot, 1, c, o, :] = jnp.concatenate([kr * hi0 + ki * hr0, kr * hi + ki * hr], 0).astype(BF16)
            hre[:, cs] = hr
            him[:, cs] = hi

    def ffn_pieces(b):
        f0 = pl.multiple_of(b * FC, FC)
        acts = []
        for n in range(FC // 128):
            fs = pl.ds(pl.multiple_of(f0 + n * 128, 128), 128)
            gu = []
            for w in (wg, wu):
                a = _nn(xsel[:, :D // 2], w[:D // 2, fs])
                yield
                gu.append(_rb(a - _nn(xsel[:, D // 2:], w[D // 2:, fs])))
                yield
            g, u = gu
            acts.append((_rb(g * jax.nn.sigmoid(g)) * u).astype(BF16))
        act = jnp.concatenate(acts, axis=1)
        yield
        yield
        for k in range(KD):
            ks = slice(k * 128, (k + 1) * 128)
            yacc[:, ks] += _nn(act, wd[pl.ds(f0, FC), ks])[:8]
            yield

    def hcat(slot, part, half):
        n = P // 256
        return jnp.concatenate([hb[slot, part, half * n + c] for c in range(n)], axis=1)

    def p2_block(b, slot, last=False):
        r0 = pl.multiple_of(b * T, T)
        ffn = iter(()) if last else ffn_pieces(b)
        H = P // 2
        for k in range(KD):
            ks = slice(k * 128, (k + 1) * 128)
            y = res[k, pl.ds(r0, T), :] + xnf[pl.ds(r0, T), ks].astype(F32) * dsk[:, ks]
            y = y + _nt(hcat(slot, 0, 0), cre[ks, :H])
            next(ffn, None)
            y = y - _nt(hcat(slot, 1, 0), cim[ks, :H])
            next(ffn, None)
            y = y + _nt(hcat(slot, 0, 1), cre[ks, H:])
            next(ffn, None)
            y = y - _nt(hcat(slot, 1, 1), cim[ks, H:])
            next(ffn, None)
            if not last:
                scan(b + 1, 1 - slot, k)
            car[k] = y
            for s in range(NSEG):
                stage[s, pl.ds(pl.multiple_of(b * J, J), J), ks] = car[k, pl.ds(s, J, stride=NSEG), :]
            if last and k in (5, 7):
                cols = pl.ds(0, 768) if k == 5 else pl.ds(768, 256)
                pltpu.make_async_copy(stage.at[:, pl.ds(b * J, J), cols],
                                      o_hbm.at[:, pl.ds(b * J, J), cols], sem_o.at[3]).start()
        if not last:
            o_copy(pl.multiple_of(b * J, J), J, 0).start()

    for c in range(P // 128):
        scan(0, 0, c)
    for cp in w_copies:
        cp.wait()
    jax.lax.fori_loop(0, NB - 1, lambda b, _: p2_block(b, b % 2), None)

    routed = [(t // SEG, t % SEG, yacc[k:k + 1, :] * jax.nn.sigmoid(jnp.full((1, D), m, F32)))
              for k, (t, m) in enumerate(((t1, m1), (t2, m2)))]
    JL = (NB - 1) * J
    for s, j, yk in routed:
        @pl.when(j >= JL)
        def _():
            prow = pl.ds(j * NSEG + s, 1)
            for q in range(KD):
                res[q, prow, :] = res[q, prow, :] + yk[:, q * 128:(q + 1) * 128]

    p2_block(NB - 1, (NB - 1) % 2, last=True)

    o_copy(0, JL, 0).wait()
    for s, j, yk in routed:
        @pl.when(j < JL)
        def _():
            srow = pl.ds(jnp.minimum(j, SEG - 1), 1)
            stage[s, srow, :] = stage[s, srow, :] + yk
    g1 = pl.multiple_of(routed[0][1] // 8 * 8, 8)
    g2 = pl.multiple_of(routed[1][1] // 8 * 8, 8)
    redo1 = g1 < JL
    redo2 = jnp.logical_and(g2 < JL, g2 != g1)
    pl.when(redo1)(lambda: o_copy(g1, 8, 1).start())
    pl.when(redo2)(lambda: o_copy(g2, 8, 2).start())
    pl.when(redo1)(lambda: o_copy(g1, 8, 1).wait())
    pl.when(redo2)(lambda: o_copy(g2, 8, 2).wait())
    o_copy(JL, J, 3).wait()


@jax.jit
def pallas_parallel_sum__ssm_conv_s5__moe_arch_mod__prompt_kernel(
    A_x: jax.Array,
    A_Lambda_re: jax.Array,
    A_Lambda_im: jax.Array,
    A_B_re: jax.Array,
    A_B_im: jax.Array,
    A_C_re: jax.Array,
    A_C_im: jax.Array,
    A_log_dt: jax.Array,
    A_Dskip: jax.Array,
    B_x: jax.Array,
    B_w_r: jax.Array,
    B_w_gate: jax.Array,
    B_w_up: jax.Array,
    B_w_down: jax.Array,
):
    del B_x
    Bsz, S, D = A_x.shape
    P = A_B_re.shape[0]
    F = B_w_gate.shape[1]
    assert Bsz == 1
    J, PC = 32, 256
    T = NSEG * J
    hbm = pl.BlockSpec(memory_space=pl.ANY)
    vmem = pl.BlockSpec(memory_space=pltpu.VMEM)
    out = pl.pallas_call(
        functools.partial(_kernel, J=J, PC=PC),
        in_specs=[hbm, vmem, vmem, hbm, hbm, hbm, hbm, vmem, vmem, vmem, hbm, hbm, hbm],
        out_specs=hbm,
        out_shape=jax.ShapeDtypeStruct((NSEG, S // NSEG, D), F32),
        scratch_shapes=[
            pltpu.VMEM((NSEG, S // NSEG, D), BF16),
            pltpu.VMEM((P, D), BF16), pltpu.VMEM((P, D), BF16),
            pltpu.VMEM((D, P), BF16), pltpu.VMEM((D, P), BF16),
            pltpu.VMEM((D, F), BF16), pltpu.VMEM((D, F), BF16), pltpu.VMEM((F, D), BF16),
            pltpu.VMEM((D // 128, S, 128), F32),
            pltpu.VMEM((S, P), F32), pltpu.VMEM((S, P), F32),
            pltpu.VMEM((NSEG, P), F32), pltpu.VMEM((NSEG, P), F32),
            pltpu.VMEM((2, NSEG, 128), F32), pltpu.VMEM((2, NSEG, 128), jnp.int32),
            pltpu.VMEM((D // 128, T, 128), F32),
            pltpu.VMEM((NSEG, S // NSEG, D), F32),
            pltpu.VMEM((2, T, D), BF16),
            pltpu.VMEM((2, 2, P // 128, T, 128), BF16),
            pltpu.VMEM((S, D), BF16),
            pltpu.VMEM((16, D), BF16), pltpu.VMEM((8, D), F32),
            pltpu.SemaphoreType.DMA((S // T,)),
            pltpu.SemaphoreType.DMA((2 * P // PC,)),
            pltpu.SemaphoreType.DMA((5,)),
            pltpu.SemaphoreType.DMA((4,)),
        ],
        compiler_params=pltpu.CompilerParams(vmem_limit_bytes=100 * 1024 * 1024),
    )(A_x.reshape(NSEG, S // NSEG, D), A_Lambda_re, A_Lambda_im, A_B_re, A_B_im,
      A_C_re, A_C_im, A_log_dt, A_Dskip, B_w_r, B_w_gate, B_w_up, B_w_down)
    return out.reshape(Bsz, S, D)
```

```python
import functools

import jax
import jax.numpy as jnp
import jax.experimental.pallas as pl
import jax.experimental.pallas.tpu as pltpu

F32 = jnp.float32
BF16 = jnp.bfloat16
NSEG = 8


def _rb(v):
    return v.astype(BF16).astype(F32)


def _layernorm_rows(x):
    d = x.shape[-1]
    m = jnp.sum(x, axis=-1, keepdims=True) * (1.0 / d)
    mb = _rb(m)
    xc = x - mb
    v = jnp.sum(xc * xc, axis=-1, keepdims=True) * (1.0 / d) - (m - mb) * (m - mb)
    s = _rb(jnp.sqrt(_rb(_rb(v) + 1e-5)))
    return _rb(_rb(xc) / s)


def _nt(a, b):
    return jax.lax.dot_general(a, b, (((1,), (1,)), ((), ())), preferred_element_type=F32)


def _nn(a, b):
    return jnp.dot(a, b, preferred_element_type=F32)


def _kernel(x_hbm, lre_ref, lim_ref, bre_hbm, bim_hbm, cre_hbm, cim_hbm, ldt_ref, dsk_ref,
            wr_ref, wg_hbm, wu_hbm, wd_hbm, o_hbm,
            xv, bre, bim, cre, cim, wg, wu, wd, bure, buim, hre, him, top, topi,
            car, stage, xb, hb, xnf, xsel, yacc, sem_x, sem_b, sem_w, sem_o, *, J, PC):
    S, D = xnf.shape
    KD = D // 128
    P = bre.shape[0]
    F = wg.shape[1]
    SEG = S // NSEG
    NB = SEG // J
    T = NSEG * J
    NC = P // PC
    FC = F // (NB - 1)

    xw_hbm = x_hbm.bitcast(jnp.int32)
    JW = J // 2

    class x_copy:
        def __init__(self, b):
            self.b = b

        def start(self):
            for s in range(NSEG):
                pltpu.make_async_copy(xw_hbm.at[s, pl.ds(self.b * JW, JW), :],
                                      xv.at[pl.ds(self.b * JW, JW), s, :], sem_x.at[self.b]).start()

        def wait(self):
            blk = xv.at[pl.ds(self.b * JW, JW)]
            pltpu.make_async_copy(blk, blk, sem_x.at[self.b]).wait()

    def steps(w):
        return jnp.concatenate([pltpu.bitcast(w << 16, F32), pltpu.bitcast(w & -65536, F32)], axis=0)

    def b_copy(c, src, dst, k):
        return pltpu.make_async_copy(
            src.at[pl.ds(c * PC, PC), :], dst.at[pl.ds(c * PC, PC), :], sem_b.at[2 * c + k])

    w_copies = [pltpu.make_async_copy(s_, d_, sem_w.at[i]) for i, (s_, d_) in enumerate(
        ((cre_hbm, cre), (cim_hbm, cim), (wg_hbm, wg), (wu_hbm, wu), (wd_hbm, wd)))]

    def o_copy(j0, n, k):
        return pltpu.make_async_copy(
            stage.at[:, pl.ds(j0, n), :], o_hbm.at[:, pl.ds(j0, n), :], sem_o.at[k])

    x_copy(0).start()
    x_copy(1).start()
    b_copy(0, bre_hbm, bre, 0).start()
    b_copy(0, bim_hbm, bim, 1).start()

    row = lambda r: r[...].astype(F32).reshape(1, -1)
    lre, lim = row(lre_ref), row(lim_ref)
    dt = _rb(jnp.exp(row(ldt_ref)))
    mag = jnp.exp(dt * lre)
    are = mag * jnp.cos(dt * lim)
    aim = mag * jnp.sin(dt * lim)
    den = lre * lre + lim * lim
    kre8 = jnp.broadcast_to(2.0 * ((are - 1.0) * lre + aim * lim) / den, (NSEG, P))
    kim8 = jnp.broadcast_to(2.0 * (aim * lre - (are - 1.0) * lim) / den, (NSEG, P))
    are8 = jnp.broadcast_to(are, (NSEG, P))
    aim8 = jnp.broadcast_to(aim, (NSEG, P))
    dsk = 1.0 + row(dsk_ref)
    wr = row(wr_ref)

    hre[...] = jnp.zeros_like(hre)
    him[...] = jnp.zeros_like(him)
    yacc[...] = jnp.zeros_like(yacc)

    JP = 16
    TP = JP * NSEG
    subd = jax.lax.broadcasted_iota(jnp.int32, (NSEG, 128), 0)
    top[0] = jnp.full((NSEG, 128), -jnp.inf, F32)
    top[1] = jnp.full((NSEG, 128), -jnp.inf, F32)
    topi[0] = subd * SEG
    topi[1] = subd * SEG + 1

    def norm(b, slot, g):
        rows = pl.ds(pl.multiple_of(b * T + g * 16, 16), 16)
        x = steps(xv[b * JW + g])
        xn = _layernorm_rows(x)
        xb[slot, g * 16:(g + 1) * 16, :] = xn.astype(BF16)
        xnf[rows, :] = xn.astype(BF16)
        r = jnp.broadcast_to(_rb(jnp.sum(xn * wr, axis=-1, keepdims=True)), (16, 128))
        b1, b2, i1, i2 = top[0], top[1], topi[0], topi[1]
        for j in range(2):
            rj = r[j * NSEG:(j + 1) * NSEG]
            tj = subd * SEG + (b * J + 2 * g + j)
            g1, g2 = rj > b1, rj > b2
            b2, i2 = jnp.where(g1, b1, jnp.where(g2, rj, b2)), jnp.where(g1, i1, jnp.where(g2, tj, i2))
            b1, i1 = jnp.where(g1, rj, b1), jnp.where(g1, tj, i1)
        top[0], top[1], topi[0], topi[1] = b1, b2, i1, i2

    def p1_block(b, slot, first=False, last=False):
        r0 = pl.multiple_of(b * T, T)
        NT = P // 128
        for c in range(NT):
            cs = slice(c * 128, (c + 1) * 128)
            if first and c % (NT // NC) == 0:
                cc = c // (NT // NC)
                b_copy(cc, bre_hbm, bre, 0).wait()
                b_copy(cc, bim_hbm, bim, 1).wait()
                if cc + 2 < NC:
                    b_copy(cc + 2, bre_hbm, bre, 0).start()
                    b_copy(cc + 2, bim_hbm, bim, 1).start()
                elif cc + 2 == NC:
                    x_copy(2).start()
            us = []
            for part, (w, bu) in enumerate(((bre, bure), (bim, buim))):
                u = _nt(xb[slot], w[cs, :])
                bu[pl.ds(r0, T), cs] = u
                us.append(u)
                if not last:
                    g = 2 * c + part
                    norm(b + 1, 1 - slot, g)
                else:
                    xb[1 - slot, :16, :256] = jnp.zeros((16, 256), BF16)
            ure, uim = us
            ar, ai = are8[:, cs], aim8[:, cs]
            hr, hi = hre[:, cs], him[:, cs]
            for j in range(J):
                js = slice(j * NSEG, (j + 1) * NSEG)
                hr, hi = (ar * hr + ure[js]) - ai * hi, (ar * hi + uim[js]) + ai * hr
            hre[:, cs] = hr
            him[:, cs] = hi

    x_copy(0).wait()
    b_copy(1, bre_hbm, bre, 0).start()
    b_copy(1, bim_hbm, bim, 1).start()
    for g in range(T // 16):
        norm(0, 0, g)
    x_copy(1).wait()
    p1_block(0, 0, first=True)
    for b in range(3, NB):
        x_copy(b).start()
    for cp in w_copies:
        cp.start()

    def p1_step(b, _):
        x_copy(b + 1).wait()
        p1_block(b, b % 2)

    jax.lax.fori_loop(1, NB - 1, p1_step, None)
    b1, b2, i1, i2 = top[0], top[1], topi[0], topi[1]
    m1 = jnp.max(b1)
    t1 = jnp.min(jnp.where(b1 == m1, i1, S))
    b1, i1 = jnp.where(i1 == t1, b2, b1), jnp.where(i1 == t1, i2, i1)
    m2 = jnp.max(b1)
    t2 = jnp.min(jnp.where(b1 == m2, i1, S))
    t1 = jnp.clip(t1, 0, S - 1)
    t2 = jnp.clip(t2, 0, S - 1)
    sub16 = jax.lax.broadcasted_iota(jnp.int32, (16, D), 0)

    def pick(t):
        s, j = t // SEG, t % SEG
        xn = _layernorm_rows(steps(xv[j // 2]))
        return jnp.sum(jnp.where(sub16 == (j % 2) * NSEG + s, xn, 0.0), axis=0, keepdims=True)

    xs = jnp.where(sub16 == 0, pick(t1), jnp.where(sub16 == 1, pick(t2), 0.0))
    xsel[:, :D // 2] = xs[:, :D // 2].astype(BF16)
    xsel[:, D // 2:] = (-xs[:, D // 2:]).astype(BF16)

    p1_block(NB - 1, (NB - 1) % 2, last=True)

    pr, pi = are8, aim8
    for _ in range(SEG.bit_length() - 1):
        pr, pi = pr * pr - pi * pi, 2.0 * pr * pi
    sub = jax.lax.broadcasted_iota(jnp.int32, (NSEG, P), 0)
    er, ei = hre[...], him[...]
    sh = 1
    while sh < NSEG:
        tr = jnp.where(sub >= sh, pltpu.roll(er, sh, 0), 0.0)
        ti = jnp.where(sub >= sh, pltpu.roll(ei, sh, 0), 0.0)
        er, ei = er + (pr * tr - pi * ti), ei + (pr * ti + pi * tr)
        pr, pi = pr * pr - pi * pi, 2.0 * pr * pi
        sh *= 2
    hre[...] = jnp.where(sub >= 1, pltpu.roll(er, 1, 0), 0.0)
    him[...] = jnp.where(sub >= 1, pltpu.roll(ei, 1, 0), 0.0)

    def scan(b, slot, c):
        r0 = pl.multiple_of(b * T, T)
        if True:
            cs = slice(c * 128, (c + 1) * 128)
            ar, ai, kr, ki = are8[:, cs], aim8[:, cs], kre8[:, cs], kim8[:, cs]
            hr, hi = hre[:, cs], him[:, cs]
            for j in range(0, J, 2):
                rows = pl.ds(pl.multiple_of(r0 + j * NSEG, 16), 16)
                ur, ui = bure[rows, cs], buim[rows, cs]
                hr0, hi0 = (ar * hr + ur[:8]) - ai * hi, (ar * hi + ui[:8]) + ai * hr
                hr, hi = (ar * hr0 + ur[8:]) - ai * hi0, (ar * hi0 + ui[8:]) + ai * hr0
                o = slice(j * NSEG, (j + 2) * NSEG)
                hb[slot, 0, c, o, :] = jnp.concatenate([kr * hr0 - ki * hi0, kr * hr - ki * hi], 0).astype(BF16)
                hb[slot, 1, c, o, :] = jnp.concatenate([kr * hi0 + ki * hr0, kr * hi + ki * hr], 0).astype(BF16)
            hre[:, cs] = hr
            him[:, cs] = hi

    def ffn_pieces(b):
        f0 = pl.multiple_of(b * FC, FC)
        acts = []
        for n in range(FC // 128):
            fs = pl.ds(pl.multiple_of(f0 + n * 128, 128), 128)
            gu = []
            for w in (wg, wu):
                a = _nn(xsel[:, :D // 2], w[:D // 2, fs])
                yield
                gu.append(_rb(a - _nn(xsel[:, D // 2:], w[D // 2:, fs])))
                yield
            g, u = gu
            acts.append((_rb(g * jax.nn.sigmoid(g)) * u).astype(BF16))
        act = jnp.concatenate(acts, axis=1)
        yield
        yield
        for k in range(KD):
            ks = slice(k * 128, (k + 1) * 128)
            yacc[:, ks] += _nn(act, wd[pl.ds(f0, FC), ks])[:8]
            yield

    def hcat(slot, part, half):
        n = P // 256
        return jnp.concatenate([hb[slot, part, half * n + c] for c in range(n)], axis=1)

    def p2_block(b, slot, last=False):
        r0 = pl.multiple_of(b * T, T)
        ffn = iter(()) if last else ffn_pieces(b)
        H = P // 2
        for k in range(KD):
            ks = slice(k * 128, (k + 1) * 128)
            y = jnp.concatenate([steps(xv[b * JW + g, :, ks]) for g in range(JW)], axis=0) + xnf[pl.ds(r0, T), ks].astype(F32) * dsk[:, ks]
            y = y + _nt(hcat(slot, 0, 0), cre[ks, :H])
            next(ffn, None)
            y = y - _nt(hcat(slot, 1, 0), cim[ks, :H])
            next(ffn, None)
            y = y + _nt(hcat(slot, 0, 1), cre[ks, H:])
            next(ffn, None)
            y = y - _nt(hcat(slot, 1, 1), cim[ks, H:])
            next(ffn, None)
            if not last:
                scan(b + 1, 1 - slot, k)
            if last:
                for s, j, yk in routed:
                    y = y + jnp.where(trow == (j - JL) * NSEG + s, yk[:, ks], 0.0)
            car[k] = y
            for s in range(NSEG):
                stage[s, pl.ds(pl.multiple_of(b * J, J), J), ks] = car[k, pl.ds(s, J, stride=NSEG), :]
            if last and k in (5, 7):
                cols = pl.ds(0, 768) if k == 5 else pl.ds(768, 256)
                pltpu.make_async_copy(stage.at[:, pl.ds(b * J, J), cols],
                                      o_hbm.at[:, pl.ds(b * J, J), cols], sem_o.at[3]).start()
        if not last:
            o_copy(pl.multiple_of(b * J, J), J, 0).start()

    for c in range(P // 128):
        scan(0, 0, c)
    for cp in w_copies:
        cp.wait()
    jax.lax.fori_loop(0, NB - 1, lambda b, _: p2_block(b, b % 2), None)

    routed = [(t // SEG, t % SEG, yacc[k:k + 1, :] * jax.nn.sigmoid(jnp.full((1, D), m, F32)))
              for k, (t, m) in enumerate(((t1, m1), (t2, m2)))]
    JL = (NB - 1) * J
    trow = jax.lax.broadcasted_iota(jnp.int32, (T, 128), 0)

    p2_block(NB - 1, (NB - 1) % 2, last=True)

    o_copy(0, JL, 0).wait()
    for s, j, yk in routed:
        @pl.when(j < JL)
        def _():
            srow = pl.ds(jnp.minimum(j, SEG - 1), 1)
            stage[s, srow, :] = stage[s, srow, :] + yk
    g1 = pl.multiple_of(routed[0][1] // 8 * 8, 8)
    g2 = pl.multiple_of(routed[1][1] // 8 * 8, 8)
    redo1 = g1 < JL
    redo2 = jnp.logical_and(g2 < JL, g2 != g1)
    pl.when(redo1)(lambda: o_copy(g1, 8, 1).start())
    pl.when(redo2)(lambda: o_copy(g2, 8, 2).start())
    pl.when(redo1)(lambda: o_copy(g1, 8, 1).wait())
    pl.when(redo2)(lambda: o_copy(g2, 8, 2).wait())
    o_copy(JL, J, 3).wait()


@jax.jit
def pallas_parallel_sum__ssm_conv_s5__moe_arch_mod__prompt_kernel(
    A_x: jax.Array,
    A_Lambda_re: jax.Array,
    A_Lambda_im: jax.Array,
    A_B_re: jax.Array,
    A_B_im: jax.Array,
    A_C_re: jax.Array,
    A_C_im: jax.Array,
    A_log_dt: jax.Array,
    A_Dskip: jax.Array,
    B_x: jax.Array,
    B_w_r: jax.Array,
    B_w_gate: jax.Array,
    B_w_up: jax.Array,
    B_w_down: jax.Array,
):
    del B_x
    Bsz, S, D = A_x.shape
    P = A_B_re.shape[0]
    F = B_w_gate.shape[1]
    assert Bsz == 1
    J, PC = 32, 256
    T = NSEG * J
    hbm = pl.BlockSpec(memory_space=pl.ANY)
    vmem = pl.BlockSpec(memory_space=pltpu.VMEM)
    out = pl.pallas_call(
        functools.partial(_kernel, J=J, PC=PC),
        in_specs=[hbm, vmem, vmem, hbm, hbm, hbm, hbm, vmem, vmem, vmem, hbm, hbm, hbm],
        out_specs=hbm,
        out_shape=jax.ShapeDtypeStruct((NSEG, S // NSEG, D), F32),
        scratch_shapes=[
            pltpu.VMEM((S // NSEG // 2, NSEG, D), jnp.int32),
            pltpu.VMEM((P, D), BF16), pltpu.VMEM((P, D), BF16),
            pltpu.VMEM((D, P), BF16), pltpu.VMEM((D, P), BF16),
            pltpu.VMEM((D, F), BF16), pltpu.VMEM((D, F), BF16), pltpu.VMEM((F, D), BF16),
            pltpu.VMEM((S, P), F32), pltpu.VMEM((S, P), F32),
            pltpu.VMEM((NSEG, P), F32), pltpu.VMEM((NSEG, P), F32),
            pltpu.VMEM((2, NSEG, 128), F32), pltpu.VMEM((2, NSEG, 128), jnp.int32),
            pltpu.VMEM((D // 128, T, 128), F32),
            pltpu.VMEM((NSEG, S // NSEG, D), F32),
            pltpu.VMEM((2, T, D), BF16),
            pltpu.VMEM((2, 2, P // 128, T, 128), BF16),
            pltpu.VMEM((S, D), BF16),
            pltpu.VMEM((16, D), BF16), pltpu.VMEM((8, D), F32),
            pltpu.SemaphoreType.DMA((S // T,)),
            pltpu.SemaphoreType.DMA((2 * P // PC,)),
            pltpu.SemaphoreType.DMA((5,)),
            pltpu.SemaphoreType.DMA((4,)),
        ],
        compiler_params=pltpu.CompilerParams(vmem_limit_bytes=100 * 1024 * 1024),
    )(A_x.reshape(NSEG, S // NSEG, D), A_Lambda_re, A_Lambda_im, A_B_re, A_B_im,
      A_C_re, A_C_im, A_log_dt, A_Dskip, B_w_r, B_w_gate, B_w_up, B_w_down)
    return out.reshape(Bsz, S, D)
```

```python
import functools

import jax
import jax.numpy as jnp
import jax.experimental.pallas as pl
import jax.experimental.pallas.tpu as pltpu

F32 = jnp.float32
BF16 = jnp.bfloat16
NSEG = 8


def _rb(v):
    return v.astype(BF16).astype(F32)


def _layernorm_rows(x):
    d = x.shape[-1]
    m = jnp.sum(x, axis=-1, keepdims=True) * (1.0 / d)
    mb = _rb(m)
    xc = x - mb
    v = jnp.sum(xc * xc, axis=-1, keepdims=True) * (1.0 / d) - (m - mb) * (m - mb)
    s = _rb(jnp.sqrt(_rb(_rb(v) + 1e-5)))
    return _rb(_rb(xc) / s)


def _nt(a, b):
    return jax.lax.dot_general(a, b, (((1,), (1,)), ((), ())), preferred_element_type=F32)


def _nn(a, b):
    return jnp.dot(a, b, preferred_element_type=F32)


def _kernel(x_hbm, lre_ref, lim_ref, bre_hbm, bim_hbm, cre_hbm, cim_hbm, ldt_ref, dsk_ref,
            wr_ref, wg_hbm, wu_hbm, wd_hbm, o_hbm,
            xv, bre, bim, cre, cim, wg, wu, wd, bure, buim, hre, him, top, topi,
            car, stage, xb, hb, xnf, xsel, yacc, sem_x, sem_b, sem_w, sem_o, *, J, PC):
    S, D = xnf.shape
    KD = D // 128
    P = bre.shape[0]
    F = wg.shape[1]
    SEG = S // NSEG
    NB = SEG // J
    T = NSEG * J
    NC = P // PC
    FC = F // (NB - 1)

    xw_hbm = x_hbm.bitcast(jnp.int32)
    JW = J // 2

    class x_copy:
        def __init__(self, b, n=1):
            self.rows, self.sem = pl.ds(b * JW, n * JW), sem_x.at[b]

        def start(self):
            for s in range(NSEG):
                pltpu.make_async_copy(xw_hbm.at[s, self.rows, :],
                                      xv.at[self.rows, s, :], self.sem).start()

        def wait(self):
            blk = xv.at[self.rows]
            pltpu.make_async_copy(blk, blk, self.sem).wait()

    def steps(w):
        return jnp.concatenate([pltpu.bitcast(w << 16, F32), pltpu.bitcast(w & -65536, F32)], axis=0)

    def b_copy(c, src, dst, k):
        return pltpu.make_async_copy(
            src.at[pl.ds(c * PC, PC), :], dst.at[pl.ds(c * PC, PC), :], sem_b.at[2 * c + k])

    w_copies = [pltpu.make_async_copy(s_, d_, sem_w.at[i]) for i, (s_, d_) in enumerate(
        ((cre_hbm, cre), (cim_hbm, cim), (wg_hbm, wg), (wu_hbm, wu), (wd_hbm, wd)))]

    def o_copy(j0, n, k):
        return pltpu.make_async_copy(
            stage.at[:, pl.ds(j0, n), :], o_hbm.at[:, pl.ds(j0, n), :], sem_o.at[k])

    x_copy(0).start()
    b_copy(0, bre_hbm, bre, 0).start()
    b_copy(0, bim_hbm, bim, 1).start()
    b_copy(1, bre_hbm, bre, 0).start()
    b_copy(1, bim_hbm, bim, 1).start()

    row = lambda r: r[...].astype(F32).reshape(1, -1)
    lre, lim = row(lre_ref), row(lim_ref)
    dt = _rb(jnp.exp(row(ldt_ref)))
    mag = jnp.exp(dt * lre)
    are = mag * jnp.cos(dt * lim)
    aim = mag * jnp.sin(dt * lim)
    den = lre * lre + lim * lim
    kre8 = jnp.broadcast_to(2.0 * ((are - 1.0) * lre + aim * lim) / den, (NSEG, P))
    kim8 = jnp.broadcast_to(2.0 * (aim * lre - (are - 1.0) * lim) / den, (NSEG, P))
    are8 = jnp.broadcast_to(are, (NSEG, P))
    aim8 = jnp.broadcast_to(aim, (NSEG, P))
    dsk = 1.0 + row(dsk_ref)
    wr = row(wr_ref)

    hre[...] = jnp.zeros_like(hre)
    him[...] = jnp.zeros_like(him)
    yacc[...] = jnp.zeros_like(yacc)

    JP = 16
    TP = JP * NSEG
    subd = jax.lax.broadcasted_iota(jnp.int32, (NSEG, 128), 0)
    top[0] = jnp.full((NSEG, 128), -jnp.inf, F32)
    top[1] = jnp.full((NSEG, 128), -jnp.inf, F32)
    topi[0] = subd * SEG
    topi[1] = subd * SEG + 1

    def norm(b, slot, g):
        rows = pl.ds(pl.multiple_of(b * T + g * 16, 16), 16)
        x = steps(xv[b * JW + g])
        xn = _layernorm_rows(x)
        xb[slot, g * 16:(g + 1) * 16, :] = xn.astype(BF16)
        xnf[rows, :] = xn.astype(BF16)
        r = jnp.broadcast_to(_rb(jnp.sum(xn * wr, axis=-1, keepdims=True)), (16, 128))
        b1, b2, i1, i2 = top[0], top[1], topi[0], topi[1]
        for j in range(2):
            rj = r[j * NSEG:(j + 1) * NSEG]
            tj = subd * SEG + (b * J + 2 * g + j)
            g1, g2 = rj > b1, rj > b2
            b2, i2 = jnp.where(g1, b1, jnp.where(g2, rj, b2)), jnp.where(g1, i1, jnp.where(g2, tj, i2))
            b1, i1 = jnp.where(g1, rj, b1), jnp.where(g1, tj, i1)
        top[0], top[1], topi[0], topi[1] = b1, b2, i1, i2

    def p1_block(b, slot, first=False, last=False):
        r0 = pl.multiple_of(b * T, T)
        NT = P // 128
        for c in range(NT):
            cs = slice(c * 128, (c + 1) * 128)
            if first and c % (NT // NC) == 0:
                cc = c // (NT // NC)
                b_copy(cc, bre_hbm, bre, 0).wait()
                b_copy(cc, bim_hbm, bim, 1).wait()
                if cc + 4 < NC:
                    b_copy(cc + 4, bre_hbm, bre, 0).start()
                    b_copy(cc + 4, bim_hbm, bim, 1).start()
                elif cc + 4 == NC:
                    x_copy(2).start()
                if cc == 0:
                    x_copy(1).start()
                if cc == NC // 2:
                    x_copy(1).wait()
            us = []
            for part, (w, bu) in enumerate(((bre, bure), (bim, buim))):
                u = _nt(xb[slot], w[cs, :])
                bu[pl.ds(r0, T), cs] = u
                us.append(u)
                if not last:
                    g = 2 * c + part
                    if not first:
                        norm(b + 1, 1 - slot, g)
                    elif g >= NT:
                        norm(b + 1, 1 - slot, 2 * (g - NT))
                        norm(b + 1, 1 - slot, 2 * (g - NT) + 1)
                else:
                    xb[1 - slot, :16, :256] = jnp.zeros((16, 256), BF16)
            ure, uim = us
            ar, ai = are8[:, cs], aim8[:, cs]
            hr, hi = hre[:, cs], him[:, cs]
            for j in range(J):
                js = slice(j * NSEG, (j + 1) * NSEG)
                hr, hi = (ar * hr + ure[js]) - ai * hi, (ar * hi + uim[js]) + ai * hr
            hre[:, cs] = hr
            him[:, cs] = hi

    x_copy(0).wait()
    for c in (2, 3):
        b_copy(c, bre_hbm, bre, 0).start()
        b_copy(c, bim_hbm, bim, 1).start()
    for g in range(T // 16):
        norm(0, 0, g)
    p1_block(0, 0, first=True)
    x_rest = x_copy(3, NB - 3)
    x_rest.start()
    for cp in w_copies[:3]:
        cp.start()

    def p1_step(b, _):
        pl.when(b == 1)(x_copy(2).wait)

        @pl.when(b == 2)
        def _():
            x_rest.wait()
            for cp in w_copies[3:]:
                cp.start()

        p1_block(b, b % 2)

    jax.lax.fori_loop(1, NB - 1, p1_step, None)
    b1, b2, i1, i2 = top[0], top[1], topi[0], topi[1]
    m1 = jnp.max(b1)
    t1 = jnp.min(jnp.where(b1 == m1, i1, S))
    b1, i1 = jnp.where(i1 == t1, b2, b1), jnp.where(i1 == t1, i2, i1)
    m2 = jnp.max(b1)
    t2 = jnp.min(jnp.where(b1 == m2, i1, S))
    t1 = jnp.clip(t1, 0, S - 1)
    t2 = jnp.clip(t2, 0, S - 1)
    sub16 = jax.lax.broadcasted_iota(jnp.int32, (16, D), 0)

    def pick(t):
        s, j = t // SEG, t % SEG
        xn = _layernorm_rows(steps(xv[j // 2]))
        return jnp.sum(jnp.where(sub16 == (j % 2) * NSEG + s, xn, 0.0), axis=0, keepdims=True)

    xs = jnp.where(sub16 == 0, pick(t1), jnp.where(sub16 == 1, pick(t2), 0.0))
    xsel[:, :D // 2] = xs[:, :D // 2].astype(BF16)
    xsel[:, D // 2:] = (-xs[:, D // 2:]).astype(BF16)

    p1_block(NB - 1, (NB - 1) % 2, last=True)

    pr, pi = are8, aim8
    for _ in range(SEG.bit_length() - 1):
        pr, pi = pr * pr - pi * pi, 2.0 * pr * pi
    sub = jax.lax.broadcasted_iota(jnp.int32, (NSEG, P), 0)
    er, ei = hre[...], him[...]
    sh = 1
    while sh < NSEG:
        tr = jnp.where(sub >= sh, pltpu.roll(er, sh, 0), 0.0)
        ti = jnp.where(sub >= sh, pltpu.roll(ei, sh, 0), 0.0)
        er, ei = er + (pr * tr - pi * ti), ei + (pr * ti + pi * tr)
        pr, pi = pr * pr - pi * pi, 2.0 * pr * pi
        sh *= 2
    hre[...] = jnp.where(sub >= 1, pltpu.roll(er, 1, 0), 0.0)
    him[...] = jnp.where(sub >= 1, pltpu.roll(ei, 1, 0), 0.0)

    def scan(b, slot, c):
        r0 = pl.multiple_of(b * T, T)
        if True:
            cs = slice(c * 128, (c + 1) * 128)
            ar, ai, kr, ki = are8[:, cs], aim8[:, cs], kre8[:, cs], kim8[:, cs]
            hr, hi = hre[:, cs], him[:, cs]
            for j in range(0, J, 2):
                rows = pl.ds(pl.multiple_of(r0 + j * NSEG, 16), 16)
                ur, ui = bure[rows, cs], buim[rows, cs]
                hr0, hi0 = (ar * hr + ur[:8]) - ai * hi, (ar * hi + ui[:8]) + ai * hr
                hr, hi = (ar * hr0 + ur[8:]) - ai * hi0, (ar * hi0 + ui[8:]) + ai * hr0
                o = slice(j * NSEG, (j + 2) * NSEG)
                hb[slot, 0, c, o, :] = jnp.concatenate([kr * hr0 - ki * hi0, kr * hr - ki * hi], 0).astype(BF16)
                hb[slot, 1, c, o, :] = jnp.concatenate([kr * hi0 + ki * hr0, kr * hi + ki * hr], 0).astype(BF16)
            hre[:, cs] = hr
            him[:, cs] = hi

    def ffn_pieces(b):
        f0 = pl.multiple_of(b * FC, FC)
        acts = []
        for n in range(FC // 128):
            fs = pl.ds(pl.multiple_of(f0 + n * 128, 128), 128)
            gu = []
            for w in (wg, wu):
                a = _nn(xsel[:, :D // 2], w[:D // 2, fs])
                yield
                gu.append(_rb(a - _nn(xsel[:, D // 2:], w[D // 2:, fs])))
                yield
            g, u = gu
            acts.append((_rb(g * jax.nn.sigmoid(g)) * u).astype(BF16))
        act = jnp.concatenate(acts, axis=1)
        yield
        yield
        for k in range(KD):
            ks = slice(k * 128, (k + 1) * 128)
            yacc[:, ks] += _nn(act, wd[pl.ds(f0, FC), ks])[:8]
            yield

    def hcat(slot, part, half):
        n = P // 256
        return jnp.concatenate([hb[slot, part, half * n + c] for c in range(n)], axis=1)

    def p2_block(b, slot, last=False):
        r0 = pl.multiple_of(b * T, T)
        ffn = iter(()) if last else ffn_pieces(b)
        H = P // 2
        for k in range(KD):
            ks = slice(k * 128, (k + 1) * 128)
            y = jnp.concatenate([steps(xv[b * JW + g, :, ks]) for g in range(JW)], axis=0) + xnf[pl.ds(r0, T), ks].astype(F32) * dsk[:, ks]
            y = y + _nt(hcat(slot, 0, 0), cre[ks, :H])
            next(ffn, None)
            y = y - _nt(hcat(slot, 1, 0), cim[ks, :H])
            next(ffn, None)
            y = y + _nt(hcat(slot, 0, 1), cre[ks, H:])
            next(ffn, None)
            y = y - _nt(hcat(slot, 1, 1), cim[ks, H:])
            next(ffn, None)
            if not last:
                scan(b + 1, 1 - slot, k)
            if last:
                for s, j, yk in routed:
                    y = y + jnp.where(trow == (j - JL) * NSEG + s, yk[:, ks], 0.0)
            car[k] = y
            for s in range(NSEG):
                stage[s, pl.ds(pl.multiple_of(b * J, J), J), ks] = car[k, pl.ds(s, J, stride=NSEG), :]
            if last and k in (5, 7):
                cols = pl.ds(0, 768) if k == 5 else pl.ds(768, 256)
                pltpu.make_async_copy(stage.at[:, pl.ds(b * J, J), cols],
                                      o_hbm.at[:, pl.ds(b * J, J), cols], sem_o.at[3]).start()
        if not last:
            o_copy(pl.multiple_of(b * J, J), J, 0).start()

    for c in range(P // 128):
        scan(0, 0, c)
    for cp in w_copies:
        cp.wait()
    jax.lax.fori_loop(0, NB - 1, lambda b, _: p2_block(b, b % 2), None)

    routed = [(t // SEG, t % SEG, yacc[k:k + 1, :] * jax.nn.sigmoid(jnp.full((1, D), m, F32)))
              for k, (t, m) in enumerate(((t1, m1), (t2, m2)))]
    JL = (NB - 1) * J
    trow = jax.lax.broadcasted_iota(jnp.int32, (T, 128), 0)

    p2_block(NB - 1, (NB - 1) % 2, last=True)

    o_copy(0, JL, 0).wait()
    for s, j, yk in routed:
        @pl.when(j < JL)
        def _():
            srow = pl.ds(jnp.minimum(j, SEG - 1), 1)
            stage[s, srow, :] = stage[s, srow, :] + yk
    g1 = pl.multiple_of(routed[0][1] // 8 * 8, 8)
    g2 = pl.multiple_of(routed[1][1] // 8 * 8, 8)
    redo1 = g1 < JL
    redo2 = jnp.logical_and(g2 < JL, g2 != g1)
    pl.when(redo1)(lambda: o_copy(g1, 8, 1).start())
    pl.when(redo2)(lambda: o_copy(g2, 8, 2).start())
    pl.when(redo1)(lambda: o_copy(g1, 8, 1).wait())
    pl.when(redo2)(lambda: o_copy(g2, 8, 2).wait())
    o_copy(JL, J, 3).wait()


@jax.jit
def pallas_parallel_sum__ssm_conv_s5__moe_arch_mod__prompt_kernel(
    A_x: jax.Array,
    A_Lambda_re: jax.Array,
    A_Lambda_im: jax.Array,
    A_B_re: jax.Array,
    A_B_im: jax.Array,
    A_C_re: jax.Array,
    A_C_im: jax.Array,
    A_log_dt: jax.Array,
    A_Dskip: jax.Array,
    B_x: jax.Array,
    B_w_r: jax.Array,
    B_w_gate: jax.Array,
    B_w_up: jax.Array,
    B_w_down: jax.Array,
):
    del B_x
    Bsz, S, D = A_x.shape
    P = A_B_re.shape[0]
    F = B_w_gate.shape[1]
    assert Bsz == 1
    J, PC = 32, 128
    T = NSEG * J
    hbm = pl.BlockSpec(memory_space=pl.ANY)
    vmem = pl.BlockSpec(memory_space=pltpu.VMEM)
    out = pl.pallas_call(
        functools.partial(_kernel, J=J, PC=PC),
        in_specs=[hbm, vmem, vmem, hbm, hbm, hbm, hbm, vmem, vmem, vmem, hbm, hbm, hbm],
        out_specs=hbm,
        out_shape=jax.ShapeDtypeStruct((NSEG, S // NSEG, D), F32),
        scratch_shapes=[
            pltpu.VMEM((S // NSEG // 2, NSEG, D), jnp.int32),
            pltpu.VMEM((P, D), BF16), pltpu.VMEM((P, D), BF16),
            pltpu.VMEM((D, P), BF16), pltpu.VMEM((D, P), BF16),
            pltpu.VMEM((D, F), BF16), pltpu.VMEM((D, F), BF16), pltpu.VMEM((F, D), BF16),
            pltpu.VMEM((S, P), F32), pltpu.VMEM((S, P), F32),
            pltpu.VMEM((NSEG, P), F32), pltpu.VMEM((NSEG, P), F32),
            pltpu.VMEM((2, NSEG, 128), F32), pltpu.VMEM((2, NSEG, 128), jnp.int32),
            pltpu.VMEM((D // 128, T, 128), F32),
            pltpu.VMEM((NSEG, S // NSEG, D), F32),
            pltpu.VMEM((2, T, D), BF16),
            pltpu.VMEM((2, 2, P // 128, T, 128), BF16),
            pltpu.VMEM((S, D), BF16),
            pltpu.VMEM((16, D), BF16), pltpu.VMEM((8, D), F32),
            pltpu.SemaphoreType.DMA((4,)),
            pltpu.SemaphoreType.DMA((2 * P // PC,)),
            pltpu.SemaphoreType.DMA((5,)),
            pltpu.SemaphoreType.DMA((4,)),
        ],
        compiler_params=pltpu.CompilerParams(vmem_limit_bytes=100 * 1024 * 1024),
    )(A_x.reshape(NSEG, S // NSEG, D), A_Lambda_re, A_Lambda_im, A_B_re, A_B_im,
      A_C_re, A_C_im, A_log_dt, A_Dskip, B_w_r, B_w_gate, B_w_up, B_w_down)
    return out.reshape(Bsz, S, D)
```

```python
import functools

import jax
import jax.numpy as jnp
import jax.experimental.pallas as pl
import jax.experimental.pallas.tpu as pltpu

F32 = jnp.float32
BF16 = jnp.bfloat16
NSEG = 8


def _rb(v):
    return v.astype(BF16).astype(F32)


def _layernorm_rows(x):
    d = x.shape[-1]
    m = jnp.sum(x, axis=-1, keepdims=True) * (1.0 / d)
    mb = _rb(m)
    xc = x - mb
    v = jnp.sum(xc * xc, axis=-1, keepdims=True) * (1.0 / d) - (m - mb) * (m - mb)
    s = _rb(jnp.sqrt(_rb(_rb(v) + 1e-5)))
    return _rb(_rb(xc) / s)


def _nt(a, b):
    return jax.lax.dot_general(a, b, (((1,), (1,)), ((), ())), preferred_element_type=F32)


def _nn(a, b):
    return jnp.dot(a, b, preferred_element_type=F32)


def _kernel(x_hbm, lre_ref, lim_ref, bre_hbm, bim_hbm, cre_hbm, cim_hbm, ldt_ref, dsk_ref,
            wr_ref, wg_hbm, wu_hbm, wd_hbm, o_hbm,
            xv, bre, bim, cre, cim, wg, wu, wd, bure, buim, hre, him, top, topi,
            car, stage, tail, xb, hb, xnf, xsel, yacc, sem_x, sem_b, sem_w, sem_o, *, J, PC):
    S, D = xnf.shape
    KD = D // 128
    P = bre.shape[0]
    F = wg.shape[1]
    SEG = S // NSEG
    NB = SEG // J
    T = NSEG * J
    NC = P // PC
    FC = F // (NB - 1)

    xw_hbm = x_hbm.bitcast(jnp.int32)
    JW = J // 2

    class x_copy:
        def __init__(self, b, n=1):
            self.rows, self.sem = pl.ds(b * JW, n * JW), sem_x.at[b]

        def start(self):
            for s in range(NSEG):
                pltpu.make_async_copy(xw_hbm.at[s, self.rows, :],
                                      xv.at[self.rows, s, :], self.sem).start()

        def wait(self):
            blk = xv.at[self.rows]
            pltpu.make_async_copy(blk, blk, self.sem).wait()

    def steps(w):
        return jnp.concatenate([pltpu.bitcast(w << 16, F32), pltpu.bitcast(w & -65536, F32)], axis=0)

    def b_copy(c, src, dst, k):
        return pltpu.make_async_copy(
            src.at[pl.ds(c * PC, PC), :], dst.at[pl.ds(c * PC, PC), :], sem_b.at[2 * c + k])

    w_copies = [pltpu.make_async_copy(s_, d_, sem_w.at[i]) for i, (s_, d_) in enumerate(
        ((cre_hbm, cre), (cim_hbm, cim), (wg_hbm, wg), (wu_hbm, wu), (wd_hbm, wd)))]

    def o_copy(s, j0, n, k):
        return pltpu.make_async_copy(
            stage.at[pl.ds(j0, n), s, :], o_hbm.at[s, pl.ds(j0, n), :], sem_o.at[k])

    x_copy(0).start()
    b_copy(0, bre_hbm, bre, 0).start()
    b_copy(0, bim_hbm, bim, 1).start()
    b_copy(1, bre_hbm, bre, 0).start()
    b_copy(1, bim_hbm, bim, 1).start()

    row = lambda r: r[...].astype(F32).reshape(1, -1)
    lre, lim = row(lre_ref), row(lim_ref)
    dt = _rb(jnp.exp(row(ldt_ref)))
    mag = jnp.exp(dt * lre)
    are = mag * jnp.cos(dt * lim)
    aim = mag * jnp.sin(dt * lim)
    den = lre * lre + lim * lim
    kre8 = jnp.broadcast_to(2.0 * ((are - 1.0) * lre + aim * lim) / den, (NSEG, P))
    kim8 = jnp.broadcast_to(2.0 * (aim * lre - (are - 1.0) * lim) / den, (NSEG, P))
    are8 = jnp.broadcast_to(are, (NSEG, P))
    aim8 = jnp.broadcast_to(aim, (NSEG, P))
    dsk = 1.0 + row(dsk_ref)
    wr = row(wr_ref)

    hre[...] = jnp.zeros_like(hre)
    him[...] = jnp.zeros_like(him)
    yacc[...] = jnp.zeros_like(yacc)

    JP = 16
    TP = JP * NSEG
    subd = jax.lax.broadcasted_iota(jnp.int32, (NSEG, 128), 0)
    top[0] = jnp.full((NSEG, 128), -jnp.inf, F32)
    top[1] = jnp.full((NSEG, 128), -jnp.inf, F32)
    topi[0] = subd * SEG
    topi[1] = subd * SEG + 1

    def norm(b, slot, g):
        rows = pl.ds(pl.multiple_of(b * T + g * 16, 16), 16)
        x = steps(xv[b * JW + g])
        xn = _layernorm_rows(x)
        xb[slot, g * 16:(g + 1) * 16, :] = xn.astype(BF16)
        xnf[rows, :] = xn.astype(BF16)
        r = jnp.broadcast_to(_rb(jnp.sum(xn * wr, axis=-1, keepdims=True)), (16, 128))
        b1, b2, i1, i2 = top[0], top[1], topi[0], topi[1]
        for j in range(2):
            rj = r[j * NSEG:(j + 1) * NSEG]
            tj = subd * SEG + (b * J + 2 * g + j)
            g1, g2 = rj > b1, rj > b2
            b2, i2 = jnp.where(g1, b1, jnp.where(g2, rj, b2)), jnp.where(g1, i1, jnp.where(g2, tj, i2))
            b1, i1 = jnp.where(g1, rj, b1), jnp.where(g1, tj, i1)
        top[0], top[1], topi[0], topi[1] = b1, b2, i1, i2

    def p1_block(b, slot, first=False, last=False):
        r0 = pl.multiple_of(b * T, T)
        NT = P // 128
        for c in range(NT):
            cs = slice(c * 128, (c + 1) * 128)
            if first and c % (NT // NC) == 0:
                cc = c // (NT // NC)
                b_copy(cc, bre_hbm, bre, 0).wait()
                b_copy(cc, bim_hbm, bim, 1).wait()
                if cc + 4 < NC:
                    b_copy(cc + 4, bre_hbm, bre, 0).start()
                    b_copy(cc + 4, bim_hbm, bim, 1).start()
                elif cc + 4 == NC:
                    x_copy(2).start()
                if cc == 0:
                    x_copy(1).start()
                if cc == NC // 2:
                    x_copy(1).wait()
            us = []
            for part, (w, bu) in enumerate(((bre, bure), (bim, buim))):
                u = _nt(xb[slot], w[cs, :])
                bu[pl.ds(r0, T), cs] = u
                us.append(u)
                if not last:
                    g = 2 * c + part
                    if not first:
                        norm(b + 1, 1 - slot, g)
                    elif g >= NT:
                        norm(b + 1, 1 - slot, 2 * (g - NT))
                        norm(b + 1, 1 - slot, 2 * (g - NT) + 1)
                else:
                    xb[1 - slot, :16, :256] = jnp.zeros((16, 256), BF16)
            ure, uim = us
            ar, ai = are8[:, cs], aim8[:, cs]
            hr, hi = hre[:, cs], him[:, cs]
            for j in range(J):
                js = slice(j * NSEG, (j + 1) * NSEG)
                hr, hi = (ar * hr + ure[js]) - ai * hi, (ar * hi + uim[js]) + ai * hr
            hre[:, cs] = hr
            him[:, cs] = hi

    x_copy(0).wait()
    for c in (2, 3):
        b_copy(c, bre_hbm, bre, 0).start()
        b_copy(c, bim_hbm, bim, 1).start()
    for g in range(T // 16):
        norm(0, 0, g)
    p1_block(0, 0, first=True)
    x_rest = x_copy(3, NB - 3)
    x_rest.start()
    for cp in w_copies[:3]:
        cp.start()

    def p1_step(b, _):
        pl.when(b == 1)(x_copy(2).wait)

        @pl.when(b == 2)
        def _():
            x_rest.wait()
            for cp in w_copies[3:]:
                cp.start()

        p1_block(b, b % 2)

    jax.lax.fori_loop(1, NB - 1, p1_step, None)
    b1, b2, i1, i2 = top[0], top[1], topi[0], topi[1]
    m1 = jnp.max(b1)
    t1 = jnp.min(jnp.where(b1 == m1, i1, S))
    b1, i1 = jnp.where(i1 == t1, b2, b1), jnp.where(i1 == t1, i2, i1)
    m2 = jnp.max(b1)
    t2 = jnp.min(jnp.where(b1 == m2, i1, S))
    t1 = jnp.clip(t1, 0, S - 1)
    t2 = jnp.clip(t2, 0, S - 1)
    sub16 = jax.lax.broadcasted_iota(jnp.int32, (16, D), 0)

    def pick(t):
        s, j = t // SEG, t % SEG
        xn = _layernorm_rows(steps(xv[j // 2]))
        return jnp.sum(jnp.where(sub16 == (j % 2) * NSEG + s, xn, 0.0), axis=0, keepdims=True)

    xs = jnp.where(sub16 == 0, pick(t1), jnp.where(sub16 == 1, pick(t2), 0.0))
    xsel[:, :D // 2] = xs[:, :D // 2].astype(BF16)
    xsel[:, D // 2:] = (-xs[:, D // 2:]).astype(BF16)

    p1_block(NB - 1, (NB - 1) % 2, last=True)

    pr, pi = are8, aim8
    for _ in range(SEG.bit_length() - 1):
        pr, pi = pr * pr - pi * pi, 2.0 * pr * pi
    sub = jax.lax.broadcasted_iota(jnp.int32, (NSEG, P), 0)
    er, ei = hre[...], him[...]
    sh = 1
    while sh < NSEG:
        tr = jnp.where(sub >= sh, pltpu.roll(er, sh, 0), 0.0)
        ti = jnp.where(sub >= sh, pltpu.roll(ei, sh, 0), 0.0)
        er, ei = er + (pr * tr - pi * ti), ei + (pr * ti + pi * tr)
        pr, pi = pr * pr - pi * pi, 2.0 * pr * pi
        sh *= 2
    hre[...] = jnp.where(sub >= 1, pltpu.roll(er, 1, 0), 0.0)
    him[...] = jnp.where(sub >= 1, pltpu.roll(ei, 1, 0), 0.0)

    def scan(b, slot, c):
        r0 = pl.multiple_of(b * T, T)
        if True:
            cs = slice(c * 128, (c + 1) * 128)
            ar, ai, kr, ki = are8[:, cs], aim8[:, cs], kre8[:, cs], kim8[:, cs]
            hr, hi = hre[:, cs], him[:, cs]
            for j in range(0, J, 2):
                rows = pl.ds(pl.multiple_of(r0 + j * NSEG, 16), 16)
                ur, ui = bure[rows, cs], buim[rows, cs]
                hr0, hi0 = (ar * hr + ur[:8]) - ai * hi, (ar * hi + ui[:8]) + ai * hr
                hr, hi = (ar * hr0 + ur[8:]) - ai * hi0, (ar * hi0 + ui[8:]) + ai * hr0
                o = slice(j * NSEG, (j + 2) * NSEG)
                hb[slot, 0, c, o, :] = jnp.concatenate([kr * hr0 - ki * hi0, kr * hr - ki * hi], 0).astype(BF16)
                hb[slot, 1, c, o, :] = jnp.concatenate([kr * hi0 + ki * hr0, kr * hi + ki * hr], 0).astype(BF16)
            hre[:, cs] = hr
            him[:, cs] = hi

    def ffn_pieces(b):
        f0 = pl.multiple_of(b * FC, FC)
        acts = []
        for n in range(FC // 128):
            fs = pl.ds(pl.multiple_of(f0 + n * 128, 128), 128)
            gu = []
            for w in (wg, wu):
                a = _nn(xsel[:, :D // 2], w[:D // 2, fs])
                yield
                gu.append(_rb(a - _nn(xsel[:, D // 2:], w[D // 2:, fs])))
                yield
            g, u = gu
            acts.append((_rb(g * jax.nn.sigmoid(g)) * u).astype(BF16))
        act = jnp.concatenate(acts, axis=1)
        yield
        yield
        for k in range(KD):
            ks = slice(k * 128, (k + 1) * 128)
            yacc[:, ks] += _nn(act, wd[pl.ds(f0, FC), ks])[:8]
            yield

    def hcat(slot, part, half):
        n = P // 256
        return jnp.concatenate([hb[slot, part, half * n + c] for c in range(n)], axis=1)

    def p2_block(b, slot, last=False):
        r0 = pl.multiple_of(b * T, T)
        ffn = iter(()) if last else ffn_pieces(b)
        H = P // 2
        for k in range(KD):
            ks = slice(k * 128, (k + 1) * 128)
            y = jnp.concatenate([steps(xv[b * JW + g, :, ks]) for g in range(JW)], axis=0) + xnf[pl.ds(r0, T), ks].astype(F32) * dsk[:, ks]
            y = y + _nt(hcat(slot, 0, 0), cre[ks, :H])
            next(ffn, None)
            y = y - _nt(hcat(slot, 1, 0), cim[ks, :H])
            next(ffn, None)
            y = y + _nt(hcat(slot, 0, 1), cre[ks, H:])
            next(ffn, None)
            y = y - _nt(hcat(slot, 1, 1), cim[ks, H:])
            next(ffn, None)
            if not last:
                scan(b + 1, 1 - slot, k)
            if not last:
                stage[pl.ds(b * J, J), :, ks] = y.reshape(J, NSEG, 128)
                continue
            for s, j, yk in routed:
                y = y + jnp.where(trow == (j - JL) * NSEG + s, yk[:, ks], 0.0)
            car[k] = y
            for s in range(NSEG):
                tail[s, :, ks] = car[k, pl.ds(s, J, stride=NSEG), :]
            if k in (KD - 3, KD - 1):
                cols = pl.ds(0, D - 256) if k == KD - 3 else pl.ds(D - 256, 256)
                pltpu.make_async_copy(tail.at[:, :, cols],
                                      o_hbm.at[:, pl.ds(JL, J), cols], sem_o.at[3]).start()
        if not last:
            for s in range(NSEG):
                o_copy(s, pl.multiple_of(b * J, J), J, 0).start()

    for c in range(P // 128):
        scan(0, 0, c)
    for cp in w_copies:
        cp.wait()
    jax.lax.fori_loop(0, NB - 1, lambda b, _: p2_block(b, b % 2), None)

    routed = [(t // SEG, t % SEG, yacc[k:k + 1, :] * jax.nn.sigmoid(jnp.full((1, D), m, F32)))
              for k, (t, m) in enumerate(((t1, m1), (t2, m2)))]
    JL = (NB - 1) * J
    trow = jax.lax.broadcasted_iota(jnp.int32, (T, 128), 0)

    p2_block(NB - 1, (NB - 1) % 2, last=True)

    pltpu.make_async_copy(stage, stage, sem_o.at[0]).wait()
    sub8 = jax.lax.broadcasted_iota(jnp.int32, (NSEG, D), 0)
    for s, j, yk in routed:
        @pl.when(j < JL)
        def _():
            stage[j] = stage[j] + jnp.where(sub8 == s, yk, 0.0)
    (s1, j1, _), (s2, j2, _) = routed
    g1 = pl.multiple_of(j1 // 8 * 8, 8)
    g2 = pl.multiple_of(j2 // 8 * 8, 8)
    redo1 = g1 < JL
    redo2 = jnp.logical_and(g2 < JL, jnp.logical_or(g2 != g1, s2 != s1))
    pl.when(redo1)(lambda: o_copy(s1, g1, 8, 1).start())
    pl.when(redo2)(lambda: o_copy(s2, g2, 8, 2).start())
    pl.when(redo1)(lambda: o_copy(s1, g1, 8, 1).wait())
    pl.when(redo2)(lambda: o_copy(s2, g2, 8, 2).wait())
    pltpu.make_async_copy(tail, tail, sem_o.at[3]).wait()


@jax.jit
def pallas_parallel_sum__ssm_conv_s5__moe_arch_mod__prompt_kernel(
    A_x: jax.Array,
    A_Lambda_re: jax.Array,
    A_Lambda_im: jax.Array,
    A_B_re: jax.Array,
    A_B_im: jax.Array,
    A_C_re: jax.Array,
    A_C_im: jax.Array,
    A_log_dt: jax.Array,
    A_Dskip: jax.Array,
    B_x: jax.Array,
    B_w_r: jax.Array,
    B_w_gate: jax.Array,
    B_w_up: jax.Array,
    B_w_down: jax.Array,
):
    del B_x
    Bsz, S, D = A_x.shape
    P = A_B_re.shape[0]
    F = B_w_gate.shape[1]
    assert Bsz == 1
    J, PC = 32, 128
    T = NSEG * J
    hbm = pl.BlockSpec(memory_space=pl.ANY)
    vmem = pl.BlockSpec(memory_space=pltpu.VMEM)
    out = pl.pallas_call(
        functools.partial(_kernel, J=J, PC=PC),
        in_specs=[hbm, vmem, vmem, hbm, hbm, hbm, hbm, vmem, vmem, vmem, hbm, hbm, hbm],
        out_specs=hbm,
        out_shape=jax.ShapeDtypeStruct((NSEG, S // NSEG, D), F32),
        scratch_shapes=[
            pltpu.VMEM((S // NSEG // 2, NSEG, D), jnp.int32),
            pltpu.VMEM((P, D), BF16), pltpu.VMEM((P, D), BF16),
            pltpu.VMEM((D, P), BF16), pltpu.VMEM((D, P), BF16),
            pltpu.VMEM((D, F), BF16), pltpu.VMEM((D, F), BF16), pltpu.VMEM((F, D), BF16),
            pltpu.VMEM((S, P), F32), pltpu.VMEM((S, P), F32),
            pltpu.VMEM((NSEG, P), F32), pltpu.VMEM((NSEG, P), F32),
            pltpu.VMEM((2, NSEG, 128), F32), pltpu.VMEM((2, NSEG, 128), jnp.int32),
            pltpu.VMEM((D // 128, T, 128), F32),
            pltpu.VMEM((S // NSEG - J, NSEG, D), F32),
            pltpu.VMEM((NSEG, J, D), F32),
            pltpu.VMEM((2, T, D), BF16),
            pltpu.VMEM((2, 2, P // 128, T, 128), BF16),
            pltpu.VMEM((S, D), BF16),
            pltpu.VMEM((16, D), BF16), pltpu.VMEM((8, D), F32),
            pltpu.SemaphoreType.DMA((4,)),
            pltpu.SemaphoreType.DMA((2 * P // PC,)),
            pltpu.SemaphoreType.DMA((5,)),
            pltpu.SemaphoreType.DMA((4,)),
        ],
        compiler_params=pltpu.CompilerParams(vmem_limit_bytes=100 * 1024 * 1024),
    )(A_x.reshape(NSEG, S // NSEG, D), A_Lambda_re, A_Lambda_im, A_B_re, A_B_im,
      A_C_re, A_C_im, A_log_dt, A_Dskip, B_w_r, B_w_gate, B_w_up, B_w_down)
    return out.reshape(Bsz, S, D)
```

```python
import functools
import itertools

import jax
import jax.numpy as jnp
import jax.experimental.pallas as pl
import jax.experimental.pallas.tpu as pltpu

F32 = jnp.float32
BF16 = jnp.bfloat16
NSEG = 8


def _rb(v):
    return v.astype(BF16).astype(F32)


def _layernorm_rows(x):
    d = x.shape[-1]
    m = jnp.sum(x, axis=-1, keepdims=True) * (1.0 / d)
    mb = _rb(m)
    xc = x - mb
    v = jnp.sum(xc * xc, axis=-1, keepdims=True) * (1.0 / d) - (m - mb) * (m - mb)
    s = _rb(jnp.sqrt(_rb(_rb(v) + 1e-5)))
    return _rb(_rb(xc) / s)


def _nt(a, b):
    return jax.lax.dot_general(a, b, (((1,), (1,)), ((), ())), preferred_element_type=F32)


def _nn(a, b):
    return jnp.dot(a, b, preferred_element_type=F32)


def _kernel(x_hbm, lre_ref, lim_ref, bre_hbm, bim_hbm, cre_hbm, cim_hbm, ldt_ref, dsk_ref,
            wr_ref, wg_hbm, wu_hbm, wd_hbm, o_hbm,
            xv, bre, bim, cre, cim, wg, wu, wd, bure, buim, hre, him, top, topi,
            car, stage, tail, xb, hb, xnf, slots, ws, xsel, yacc, sem_x, sem_b, sem_w, sem_o, *, J, PC):
    S, D = xnf.shape
    KD = D // 128
    P = bre.shape[0]
    F = wg.shape[1]
    SEG = S // NSEG
    NB = SEG // J
    T = NSEG * J
    NC = P // PC
    FC = F // (NB - 1)

    xw_hbm = x_hbm.bitcast(jnp.int32)
    JW = J // 2

    class x_copy:
        def __init__(self, b, n=1):
            self.rows, self.sem = pl.ds(b * JW, n * JW), sem_x.at[b]

        def start(self):
            for s in range(NSEG):
                pltpu.make_async_copy(xw_hbm.at[s, self.rows, :],
                                      xv.at[self.rows, s, :], self.sem).start()

        def wait(self):
            blk = xv.at[self.rows]
            pltpu.make_async_copy(blk, blk, self.sem).wait()

    def steps(w):
        return jnp.concatenate([pltpu.bitcast(w << 16, F32), pltpu.bitcast(w & -65536, F32)], axis=0)

    def b_copy(c, src, dst, k):
        return pltpu.make_async_copy(
            src.at[pl.ds(c * PC, PC), :], dst.at[pl.ds(c * PC, PC), :], sem_b.at[2 * c + k])

    f_lo, f_up = pl.ds(0, FC), pl.ds(FC, F - FC)
    w_copies = [pltpu.make_async_copy(s_, d_, sem_w.at[i]) for i, (s_, d_) in enumerate(
        [(cre_hbm, cre), (cim_hbm, cim)]
        + [pair for f in (f_lo, f_up) for pair in (
            (wg_hbm.at[:, f], wg.at[:, f]), (wu_hbm.at[:, f], wu.at[:, f]), (wd_hbm.at[f], wd.at[f]))])]

    def o_copy(s, j0, n, k):
        return pltpu.make_async_copy(
            stage.at[pl.ds(j0, n), s, :], o_hbm.at[s, pl.ds(j0, n), :], sem_o.at[k])

    x_copy(0).start()
    b_copy(0, bre_hbm, bre, 0).start()
    b_copy(0, bim_hbm, bim, 1).start()
    b_copy(1, bre_hbm, bre, 0).start()
    b_copy(1, bim_hbm, bim, 1).start()

    row = lambda r: r[...].astype(F32).reshape(1, -1)
    lre, lim = row(lre_ref), row(lim_ref)
    dt = _rb(jnp.exp(row(ldt_ref)))
    mag = jnp.exp(dt * lre)
    are = mag * jnp.cos(dt * lim)
    aim = mag * jnp.sin(dt * lim)
    den = lre * lre + lim * lim
    kre8 = jnp.broadcast_to(2.0 * ((are - 1.0) * lre + aim * lim) / den, (NSEG, P))
    kim8 = jnp.broadcast_to(2.0 * (aim * lre - (are - 1.0) * lim) / den, (NSEG, P))
    are8 = jnp.broadcast_to(are, (NSEG, P))
    aim8 = jnp.broadcast_to(aim, (NSEG, P))
    dsk = 1.0 + row(dsk_ref)
    wr = row(wr_ref)

    slots[0] = 0
    for c in range(P // 128):
        hre[c] = jnp.zeros((NSEG, 128), F32)
        him[c] = jnp.zeros((NSEG, 128), F32)
    yacc[...] = jnp.zeros_like(yacc)

    JP = 16
    TP = JP * NSEG
    subd = jax.lax.broadcasted_iota(jnp.int32, (NSEG, 128), 0)
    top[0] = jnp.full((NSEG, 128), -jnp.inf, F32)
    top[1] = jnp.full((NSEG, 128), -jnp.inf, F32)
    topi[0] = subd * SEG
    topi[1] = subd * SEG + 1

    def norm(b, slot, g):
        rows = pl.ds(pl.multiple_of(b * T + g * 16, 16), 16)
        x = steps(xv[b * JW + g])
        xn = _layernorm_rows(x)
        xb[slot, g * 16:(g + 1) * 16, :] = xn.astype(BF16)
        xnf[rows, :] = xn.astype(BF16)
        r = jnp.broadcast_to(_rb(jnp.sum(xn * wr, axis=-1, keepdims=True)), (16, 128))
        b1, b2, i1, i2 = top[0], top[1], topi[0], topi[1]
        for j in range(2):
            rj = r[j * NSEG:(j + 1) * NSEG]
            tj = subd * SEG + (b * J + 2 * g + j)
            g1, g2 = rj > b1, rj > b2
            b2, i2 = jnp.where(g1, b1, jnp.where(g2, rj, b2)), jnp.where(g1, i1, jnp.where(g2, tj, i2))
            b1, i1 = jnp.where(g1, rj, b1), jnp.where(g1, tj, i1)
        top[0], top[1], topi[0], topi[1] = b1, b2, i1, i2

    def weight_sums(g):
        n = D // 2 // (2 * P // 128)
        for i in range(n // 16):
            lo = pl.ds(g * n + i * 16, 16)
            up = pl.ds(D // 2 + g * n + i * 16, 16)
            for cq in range(0, P, 256):
                cc = slice(cq, cq + 256)
                w11, w12 = cre[lo, cc].astype(F32), cre[up, cc].astype(F32)
                w21, w22 = cim[lo, cc].astype(F32), cim[up, cc].astype(F32)
                for q, v in enumerate((w11 + w22, w12 - w22, w21 - w11, w11 + w12, w21 + w22)):
                    ws[q, lo, cc] = v.astype(BF16)

    def p1_block(b, slot, first=False, last=False):
        r0 = pl.multiple_of(b * T, T)
        NT = P // 128
        for c in range(NT):
            cs = slice(c * 128, (c + 1) * 128)
            if first and c % (NT // NC) == 0:
                cc = c // (NT // NC)
                b_copy(cc, bre_hbm, bre, 0).wait()
                b_copy(cc, bim_hbm, bim, 1).wait()
                if cc + 4 < NC:
                    b_copy(cc + 4, bre_hbm, bre, 0).start()
                    b_copy(cc + 4, bim_hbm, bim, 1).start()
                elif cc + 4 == NC:
                    x_copy(2).start()
                if cc == 0:
                    x_copy(1).start()
                if cc == NC // 2:
                    x_copy(1).wait()
            us = []
            for part, (w, bu) in enumerate(((bre, bure), (bim, buim))):
                u = _nt(xb[slot], w[cs, :])
                if last and 2 * c + part >= 4:
                    next(last, None)
                    next(last, None)
                bu[pl.ds(r0, T), cs] = u
                us.append(u)
                if not last:
                    g = 2 * c + part
                    if not first:
                        norm(b + 1, 1 - slot, g)
                    elif g >= NT:
                        norm(b + 1, 1 - slot, 2 * (g - NT))
                        norm(b + 1, 1 - slot, 2 * (g - NT) + 1)
                    else:
                        xb[1 - slot, :16, :256] = jnp.zeros((16, 256), BF16)
                else:
                    weight_sums(2 * c + part)
                    xb[1 - slot, :16, :256] = jnp.zeros((16, 256), BF16)
            ure, uim = us
            ar, ai = are8[:, cs], aim8[:, cs]
            hr, hi = hre[c], him[c]
            for j in range(J):
                js = slice(j * NSEG, (j + 1) * NSEG)
                hr, hi = (ar * hr + ure[js]) - ai * hi, (ar * hi + uim[js]) + ai * hr
            hre[c] = hr
            him[c] = hi

    x_copy(0).wait()
    for c in (2, 3):
        b_copy(c, bre_hbm, bre, 0).start()
        b_copy(c, bim_hbm, bim, 1).start()
    for g in range(T // 16):
        norm(0, 0, g)
    p1_block(0, slots[0] % 2, first=True)
    x_rest = x_copy(3, NB - 3)
    x_rest.start()
    for cp in w_copies[:6]:
        cp.start()

    def p1_step(b, _):
        pl.when(b == 1)(x_copy(2).wait)

        @pl.when(b == 2)
        def _():
            x_rest.wait()
            for cp in w_copies[6:]:
                cp.start()

        @pl.when(b == NB - 3)
        def _():
            w_copies[0].wait()
            w_copies[1].wait()

        p1_block(b, b % 2)

    jax.lax.fori_loop(1, NB - 1, p1_step, None)
    for cp in w_copies[2:5]:
        cp.wait()

    b1, b2, i1, i2 = top[0], top[1], topi[0], topi[1]
    m1 = jnp.max(b1)
    t1 = jnp.min(jnp.where(b1 == m1, i1, S))
    b1, i1 = jnp.where(i1 == t1, b2, b1), jnp.where(i1 == t1, i2, i1)
    m2 = jnp.max(b1)
    t2 = jnp.min(jnp.where(b1 == m2, i1, S))
    t1 = jnp.clip(t1, 0, S - 1)
    t2 = jnp.clip(t2, 0, S - 1)
    sub16 = jax.lax.broadcasted_iota(jnp.int32, (16, D), 0)

    def pick(t):
        s, j = t // SEG, t % SEG
        xn = _layernorm_rows(steps(xv[j // 2]))
        return jnp.sum(jnp.where(sub16 == (j % 2) * NSEG + s, xn, 0.0), axis=0, keepdims=True)

    xs = jnp.where(sub16 == 0, pick(t1), jnp.where(sub16 == 1, pick(t2), 0.0))
    xsel[:, :D // 2] = xs[:, :D // 2].astype(BF16)
    xsel[:, D // 2:] = (-xs[:, D // 2:]).astype(BF16)

    def ffn_pieces(b):
        f0 = pl.multiple_of(b * FC, FC) if not isinstance(b, int) else b * FC
        acts = []
        for n in range(FC // 128):
            fs = pl.ds(pl.multiple_of(f0 + n * 128, 128), 128)
            gu = []
            for w in (wg, wu):
                a = _nn(xsel[:, :D // 2], w[:D // 2, fs])
                yield
                gu.append(_rb(a - _nn(xsel[:, D // 2:], w[D // 2:, fs])))
                yield
            g, u = gu
            acts.append((_rb(g * jax.nn.sigmoid(g)) * u).astype(BF16))
        act = jnp.concatenate(acts, axis=1)
        for k in range(KD):
            ks = slice(k * 128, (k + 1) * 128)
            yacc[:, ks] += _nn(act, wd[pl.ds(f0, FC), ks])[:8]
            yield

    p1_block(NB - 1, (slots[0] + NB - 1) % 2, last=ffn_pieces(0))

    pr, pi = are8, aim8
    for _ in range(SEG.bit_length() - 1):
        pr, pi = pr * pr - pi * pi, 2.0 * pr * pi
    sub = jax.lax.broadcasted_iota(jnp.int32, (NSEG, P), 0)
    er = jnp.concatenate([hre[c] for c in range(P // 128)], axis=1)
    ei = jnp.concatenate([him[c] for c in range(P // 128)], axis=1)
    sh = 1
    while sh < NSEG:
        tr = jnp.where(sub >= sh, pltpu.roll(er, sh, 0), 0.0)
        ti = jnp.where(sub >= sh, pltpu.roll(ei, sh, 0), 0.0)
        er, ei = er + (pr * tr - pi * ti), ei + (pr * ti + pi * tr)
        pr, pi = pr * pr - pi * pi, 2.0 * pr * pi
        sh *= 2
    er = jnp.where(sub >= 1, pltpu.roll(er, 1, 0), 0.0)
    ei = jnp.where(sub >= 1, pltpu.roll(ei, 1, 0), 0.0)

    J2 = 2 * J
    T2 = NSEG * J2
    NB2 = SEG // J2
    DH = D // 2

    def scan(b, slot, c, init=None):
        cs = slice(c * 128, (c + 1) * 128)
        ar, ai, kr, ki = are8[:, cs], aim8[:, cs], kre8[:, cs], kim8[:, cs]
        nkr = -kr
        hr, hi = init or (hre[c], him[c])
        for j in range(0, J2, 4):
            ops = []
            for jj in (j, j + 2):
                h = []
                for step in (jj, jj + 1):
                    rows = pl.ds(pl.multiple_of(b * T2 + step * NSEG, NSEG), NSEG)
                    hr, hi = (ar * hr + bure[rows, cs]) - ai * hi, (ar * hi + buim[rows, cs]) + ai * hr
                    h += [kr * hr - ki * hi, nkr * hi - ki * hr]
                h11, h12, h21, h22 = h
                ops.append((h11 + h22, h21 + h22, h11, h22, h11 + h12, h21 - h11, h12 - h22))
            o = slice(j * NSEG // 2, j * NSEG // 2 + 16)
            for i in range(7):
                hb[slot, i, c, o, :] = jnp.concatenate([ops[0][i], ops[1][i]], 0).astype(BF16)
            if j + 4 == J2:
                hre[c] = hr
                him[c] = hi
            if (j + 4) % (J2 // 4) == 0:
                yield

    def p2_block(b, slot, last=False):
        ffn = iter(()) if last else itertools.chain(ffn_pieces(2 * b + 1), ffn_pieces(2 * b + 2))
        for n in range(DH // 128):
            ns = slice(n * 128, (n + 1) * 128)
            n2 = slice(DH + n * 128, DH + (n + 1) * 128)
            nxt = iter(()) if last else itertools.chain(
                scan(b + 1, 1 - slot, 2 * n), scan(b + 1, 1 - slot, 2 * n + 1))

            def prod(i, w):
                halves = []
                for half in range(2):
                    cc = range(half * (P // 256), (half + 1) * (P // 256))
                    lhs = jnp.concatenate([hb[slot, i, c] for c in cc], axis=1)
                    halves.append(_nt(lhs, w[:, half * (P // 2):(half + 1) * (P // 2)]))
                    next(ffn, None)
                next(nxt, None)
                return halves[0] + halves[1]

            def resid(ks):
                r = [steps(xv[b * J + g, :, ks])
                     + xnf[pl.ds(pl.multiple_of(b * T2 + g * 16, 16), 16), ks].astype(F32) * dsk[:, ks]
                     for g in range(J)]
                return jnp.concatenate([v[:8] for v in r], 0), jnp.concatenate([v[8:] for v in r], 0)

            y11, y21 = resid(ns)
            y12, y22 = resid(n2)
            m = prod(0, ws.at[0, ns])
            y11, y22 = y11 + m, y22 + m
            m = prod(1, cre.at[ns])
            y21, y22 = y21 + m, y22 - m
            m = prod(2, ws.at[1, ns])
            y12, y22 = y12 + m, y22 + m
            m = prod(3, ws.at[2, ns])
            y11, y21 = y11 + m, y21 + m
            m = prod(4, cim.at[n2])
            y11, y12 = y11 - m, y12 + m
            y22 = y22 + prod(5, ws.at[3, ns])
            y11 = y11 + prod(6, ws.at[4, ns])
            next(nxt, None)
            for q, (ks, ya, yb) in enumerate(((ns, y11, y21), (n2, y12, y22))):
                slabs = [v[g * NSEG:(g + 1) * NSEG] for g in range(J) for v in (ya, yb)]
                if not last:
                    for j, v in enumerate(slabs):
                        stage[b * J2 + j, :, ks] = v
                    continue
                y = jnp.concatenate(slabs, axis=0)
                for s, j, yk in routed:
                    y = y + jnp.where(trow == (j - JL) * NSEG + s, yk[:, ks], 0.0)
                car[2 * n + q] = y
                for s in range(NSEG):
                    tail[s, :, ks] = car[2 * n + q, pl.ds(s, J2, stride=NSEG), :]
                if n >= 2:
                    cols = pl.ds(q * DH, 384) if n == 2 else ks
                    pltpu.make_async_copy(tail.at[:, :, cols],
                                          o_hbm.at[:, pl.ds(JL, J2), cols], sem_o.at[3]).start()
        if not last:
            for s in range(NSEG):
                o_copy(s, pl.multiple_of(b * J2, J2), J2, 0).start()

    for c in range(P // 128):
        cs = slice(c * 128, (c + 1) * 128)
        for _ in scan(0, 0, c, (er[:, cs], ei[:, cs])):
            pass
    for cp in w_copies[5:]:
        cp.wait()
    jax.lax.fori_loop(0, NB2 - 1, lambda b, _: p2_block(b, b % 2), None)

    routed = [(t // SEG, t % SEG, yacc[k:k + 1, :] * jax.nn.sigmoid(jnp.full((1, D), m, F32)))
              for k, (t, m) in enumerate(((t1, m1), (t2, m2)))]
    JL = SEG - J2
    trow = jax.lax.broadcasted_iota(jnp.int32, (T2, 128), 0)

    p2_block(NB2 - 1, (NB2 - 1) % 2, last=True)

    pltpu.make_async_copy(stage, stage, sem_o.at[0]).wait()
    sub8 = jax.lax.broadcasted_iota(jnp.int32, (NSEG, D), 0)
    for s, j, yk in routed:
        @pl.when(j < JL)
        def _():
            stage[j] = stage[j] + jnp.where(sub8 == s, yk, 0.0)
    (s1, j1, _), (s2, j2, _) = routed
    g1 = pl.multiple_of(j1 // 8 * 8, 8)
    g2 = pl.multiple_of(j2 // 8 * 8, 8)
    redo1 = g1 < JL
    redo2 = jnp.logical_and(g2 < JL, jnp.logical_or(g2 != g1, s2 != s1))
    pl.when(redo1)(lambda: o_copy(s1, g1, 8, 1).start())
    pl.when(redo2)(lambda: o_copy(s2, g2, 8, 2).start())
    pl.when(redo1)(lambda: o_copy(s1, g1, 8, 1).wait())
    pl.when(redo2)(lambda: o_copy(s2, g2, 8, 2).wait())
    pltpu.make_async_copy(tail, tail, sem_o.at[3]).wait()


@jax.jit
def pallas_parallel_sum__ssm_conv_s5__moe_arch_mod__prompt_kernel(
    A_x: jax.Array,
    A_Lambda_re: jax.Array,
    A_Lambda_im: jax.Array,
    A_B_re: jax.Array,
    A_B_im: jax.Array,
    A_C_re: jax.Array,
    A_C_im: jax.Array,
    A_log_dt: jax.Array,
    A_Dskip: jax.Array,
    B_x: jax.Array,
    B_w_r: jax.Array,
    B_w_gate: jax.Array,
    B_w_up: jax.Array,
    B_w_down: jax.Array,
):
    del B_x
    Bsz, S, D = A_x.shape
    P = A_B_re.shape[0]
    F = B_w_gate.shape[1]
    assert Bsz == 1
    J, PC = 32, 128
    T = NSEG * J
    hbm = pl.BlockSpec(memory_space=pl.ANY)
    vmem = pl.BlockSpec(memory_space=pltpu.VMEM)
    out = pl.pallas_call(
        functools.partial(_kernel, J=J, PC=PC),
        in_specs=[hbm, vmem, vmem, hbm, hbm, hbm, hbm, vmem, vmem, vmem, hbm, hbm, hbm],
        out_specs=hbm,
        out_shape=jax.ShapeDtypeStruct((NSEG, S // NSEG, D), F32),
        scratch_shapes=[
            pltpu.VMEM((S // NSEG // 2, NSEG, D), jnp.int32),
            pltpu.VMEM((P, D), BF16), pltpu.VMEM((P, D), BF16),
            pltpu.VMEM((D, P), BF16), pltpu.VMEM((D, P), BF16),
            pltpu.VMEM((D, F), BF16), pltpu.VMEM((D, F), BF16), pltpu.VMEM((F, D), BF16),
            pltpu.VMEM((S, P), F32), pltpu.VMEM((S, P), F32),
            pltpu.VMEM((P // 128, NSEG, 128), F32), pltpu.VMEM((P // 128, NSEG, 128), F32),
            pltpu.VMEM((2, NSEG, 128), F32), pltpu.VMEM((2, NSEG, 128), jnp.int32),
            pltpu.VMEM((D // 128, 2 * T, 128), F32),
            pltpu.VMEM((S // NSEG - 2 * J, NSEG, D), F32),
            pltpu.VMEM((NSEG, 2 * J, D), F32),
            pltpu.VMEM((2, T, D), BF16),
            pltpu.VMEM((2, 7, P // 128, T, 128), BF16),
            pltpu.VMEM((S, D), BF16), pltpu.SMEM((1,), jnp.int32), pltpu.VMEM((5, D // 2, P), BF16),
            pltpu.VMEM((16, D), BF16), pltpu.VMEM((8, D), F32),
            pltpu.SemaphoreType.DMA((4,)),
            pltpu.SemaphoreType.DMA((2 * P // PC,)),
            pltpu.SemaphoreType.DMA((8,)),
            pltpu.SemaphoreType.DMA((4,)),
        ],
        compiler_params=pltpu.CompilerParams(vmem_limit_bytes=100 * 1024 * 1024),
    )(A_x.reshape(NSEG, S // NSEG, D), A_Lambda_re, A_Lambda_im, A_B_re, A_B_im,
      A_C_re, A_C_im, A_log_dt, A_Dskip, B_w_r, B_w_gate, B_w_up, B_w_down)
    return out.reshape(Bsz, S, D)
```

```python
import itertools

import jax
import jax.numpy as jnp
import jax.experimental.pallas as pl
import jax.experimental.pallas.tpu as pltpu

F32 = jnp.float32
BF16 = jnp.bfloat16
NSEG = 8
J = 32


def _rb(v):
    return v.astype(BF16).astype(F32)


def _layernorm_rows(x):
    d = x.shape[-1]
    m = jnp.sum(x, axis=-1, keepdims=True) * (1.0 / d)
    mb = _rb(m)
    xc = x - mb
    v = jnp.sum(xc * xc, axis=-1, keepdims=True) * (1.0 / d) - (m - mb) * (m - mb)
    s = _rb(jnp.sqrt(_rb(_rb(v) + 1e-5)))
    return _rb(_rb(xc) / s)


def _steps(w):
    return jnp.concatenate([pltpu.bitcast(w << 16, F32), pltpu.bitcast(w & -65536, F32)], axis=0)


def _nt(a, b):
    return jax.lax.dot_general(a, b, (((1,), (1,)), ((), ())), preferred_element_type=F32)


def _nn(a, b):
    return jnp.dot(a, b, preferred_element_type=F32)


def _kernel(x_hbm, lre_ref, lim_ref, bre_hbm, bim_hbm, cre_hbm, cim_hbm, ldt_ref, dsk_ref,
            wr_ref, wg_hbm, wu_hbm, wd_hbm, o_hbm,
            xv, bre, bim, cre, cim, wg, wu, wd, bure, buim, hre, him, top, topi,
            car, stage, tail, xb, hb, xnf, slots, ws, xsel, yacc, sem_x, sem_b, sem_w, sem_o):
    S, D = xnf.shape
    P = bre.shape[0]
    F = wg.shape[1]
    KD, NT, DH = D // 128, P // 128, D // 2
    SEG = S // NSEG
    T, NB, JW = NSEG * J, SEG // J, J // 2
    J2 = 2 * J
    T2, NB2 = NSEG * J2, SEG // J2
    JL = SEG - J2
    FC = F // (2 * NB2 - 1)

    xw_hbm = x_hbm.bitcast(jnp.int32)

    class x_copy:
        def __init__(self, b, n=1):
            self.rows, self.sem = pl.ds(b * JW, n * JW), sem_x.at[b]

        def start(self):
            for s in range(NSEG):
                pltpu.make_async_copy(xw_hbm.at[s, self.rows, :], xv.at[self.rows, s, :], self.sem).start()

        def wait(self):
            pltpu.make_async_copy(xv.at[self.rows], xv.at[self.rows], self.sem).wait()

    def b_copies(c):
        rows = pl.ds(c * 128, 128)
        return [pltpu.make_async_copy(src.at[rows, :], dst.at[rows, :], sem_b.at[2 * c + k])
                for k, (src, dst) in enumerate(((bre_hbm, bre), (bim_hbm, bim)))]

    w_copies = [pltpu.make_async_copy(src, dst, sem_w.at[i]) for i, (src, dst) in enumerate(
        [(cre_hbm, cre), (cim_hbm, cim)]
        + [pair for f in (pl.ds(0, FC), pl.ds(FC, F - FC)) for pair in (
            (wg_hbm.at[:, f], wg.at[:, f]), (wu_hbm.at[:, f], wu.at[:, f]), (wd_hbm.at[f], wd.at[f]))])]

    def o_copy(s, j0, n, k):
        return pltpu.make_async_copy(
            stage.at[pl.ds(j0, n), s, :], o_hbm.at[s, pl.ds(j0, n), :], sem_o.at[k])

    def start(copies):
        for cp in copies:
            cp.start()

    def wait(copies):
        for cp in copies:
            cp.wait()

    x_copy(0).start()
    start(b_copies(0) + b_copies(1))

    row = lambda r: r[...].astype(F32).reshape(1, -1)
    lre, lim = row(lre_ref), row(lim_ref)
    dt = _rb(jnp.exp(row(ldt_ref)))
    mag = jnp.exp(dt * lre)
    are = mag * jnp.cos(dt * lim)
    aim = mag * jnp.sin(dt * lim)
    den = lre * lre + lim * lim
    kre8 = jnp.broadcast_to(2.0 * ((are - 1.0) * lre + aim * lim) / den, (NSEG, P))
    kim8 = jnp.broadcast_to(2.0 * (aim * lre - (are - 1.0) * lim) / den, (NSEG, P))
    are8 = jnp.broadcast_to(are, (NSEG, P))
    aim8 = jnp.broadcast_to(aim, (NSEG, P))
    dsk = 1.0 + row(dsk_ref)
    wr = row(wr_ref)

    slots[0] = 0
    for c in range(NT):
        hre[c] = jnp.zeros((NSEG, 128), F32)
        him[c] = jnp.zeros((NSEG, 128), F32)
    yacc[...] = jnp.zeros_like(yacc)
    subd = jax.lax.broadcasted_iota(jnp.int32, (NSEG, 128), 0)
    top[0] = jnp.full((NSEG, 128), -jnp.inf, F32)
    top[1] = jnp.full((NSEG, 128), -jnp.inf, F32)
    topi[0] = subd * SEG
    topi[1] = subd * SEG + 1

    def norm(b, slot, g):
        rows = pl.ds(pl.multiple_of(b * T + g * 16, 16), 16)
        xn = _layernorm_rows(_steps(xv[b * JW + g]))
        xb[slot, g * 16:(g + 1) * 16, :] = xn.astype(BF16)
        xnf[rows, :] = xn.astype(BF16)
        r = jnp.broadcast_to(_rb(jnp.sum(xn * wr, axis=-1, keepdims=True)), (16, 128))
        b1, b2, i1, i2 = top[0], top[1], topi[0], topi[1]
        for j in range(2):
            rj = r[j * NSEG:(j + 1) * NSEG]
            tj = subd * SEG + (b * J + 2 * g + j)
            g1, g2 = rj > b1, rj > b2
            b2, i2 = jnp.where(g1, b1, jnp.where(g2, rj, b2)), jnp.where(g1, i1, jnp.where(g2, tj, i2))
            b1, i1 = jnp.where(g1, rj, b1), jnp.where(g1, tj, i1)
        top[0], top[1], topi[0], topi[1] = b1, b2, i1, i2

    def weight_sums(g):
        lo = pl.ds(pl.multiple_of(g * 16, 16), 16)
        up = pl.ds(pl.multiple_of(DH + g * 16, 16), 16)
        for cq in range(0, P, 256):
            cc = slice(cq, cq + 256)
            w11, w12 = cre[lo, cc].astype(F32), cre[up, cc].astype(F32)
            w21, w22 = cim[lo, cc].astype(F32), cim[up, cc].astype(F32)
            for q, v in enumerate((w11 + w22, w12 - w22, w21 - w11, w11 + w12, w21 + w22)):
                ws[q, lo, cc] = v.astype(BF16)

    def p1_block(b, slot, first=False, ffn=None, sums=False):
        r0 = pl.multiple_of(b * T, T)
        for c in range(NT):
            cs = slice(c * 128, (c + 1) * 128)
            if first:
                wait(b_copies(c))
                if c + 4 < NT:
                    start(b_copies(c + 4))
                elif c + 4 == NT:
                    x_copy(2).start()
                if c == 0:
                    x_copy(1).start()
                if c == NT // 2:
                    x_copy(1).wait()
            us = []
            for part, (w, bu) in enumerate(((bre, bure), (bim, buim))):
                u = _nt(xb[slot], w[cs, :])
                bu[pl.ds(r0, T), cs] = u
                us.append(u)
                g = 2 * c + part
                if ffn is not None and g >= 4:
                    next(ffn, None)
                    next(ffn, None)
                if ffn is not None or (first and g < NT):
                    xb[1 - slot, :16, :256] = jnp.zeros((16, 256), BF16)
                elif first:
                    norm(b + 1, 1 - slot, 2 * (g - NT))
                    norm(b + 1, 1 - slot, 2 * (g - NT) + 1)
                else:
                    norm(b + 1, 1 - slot, g)
                    if sums and part == 1:
                        weight_sums((b - 3) * NT + c)
            ure, uim = us
            ar, ai = are8[:, cs], aim8[:, cs]
            hr, hi = hre[c], him[c]
            for j in range(J):
                js = slice(j * NSEG, (j + 1) * NSEG)
                hr, hi = (ar * hr + ure[js]) - ai * hi, (ar * hi + uim[js]) + ai * hr
            hre[c] = hr
            him[c] = hi

    x_copy(0).wait()
    start(b_copies(2) + b_copies(3))
    for g in range(T // 16):
        norm(0, 0, g)
    p1_block(0, slots[0] % 2, first=True)
    x_rest = x_copy(3, NB - 3)
    x_rest.start()
    start(w_copies[:2])

    def p1_step(b, _):
        pl.when(b == 1)(x_copy(2).wait)

        @pl.when(b == 2)
        def _():
            x_rest.wait()
            start(w_copies[2:])

        p1_block(b, b % 2)

    jax.lax.fori_loop(1, 3, p1_step, None)
    wait(w_copies[:2])
    jax.lax.fori_loop(3, NB - 1, lambda b, _: p1_block(b, b % 2, sums=True), None)
    wait(w_copies[2:5])

    b1, b2, i1, i2 = top[0], top[1], topi[0], topi[1]
    m1 = jnp.max(b1)
    t1 = jnp.min(jnp.where(b1 == m1, i1, S))
    b1, i1 = jnp.where(i1 == t1, b2, b1), jnp.where(i1 == t1, i2, i1)
    m2 = jnp.max(b1)
    t2 = jnp.min(jnp.where(b1 == m2, i1, S))
    t1 = jnp.clip(t1, 0, S - 1)
    t2 = jnp.clip(t2, 0, S - 1)
    sub16 = jax.lax.broadcasted_iota(jnp.int32, (16, D), 0)

    def pick(t):
        s, j = t // SEG, t % SEG
        xn = _layernorm_rows(_steps(xv[j // 2]))
        return jnp.sum(jnp.where(sub16 == (j % 2) * NSEG + s, xn, 0.0), axis=0, keepdims=True)

    xs = jnp.where(sub16 == 0, pick(t1), jnp.where(sub16 == 1, pick(t2), 0.0))
    xsel[:, :DH] = xs[:, :DH].astype(BF16)
    xsel[:, DH:] = (-xs[:, DH:]).astype(BF16)

    def ffn_pieces(q):
        f0 = q * FC if isinstance(q, int) else pl.multiple_of(q * FC, FC)
        acts = []
        for n in range(FC // 128):
            fs = pl.ds(pl.multiple_of(f0 + n * 128, 128), 128)
            gu = []
            for w in (wg, wu):
                a = _nn(xsel[:, :DH], w[:DH, fs])
                yield
                gu.append(_rb(a - _nn(xsel[:, DH:], w[DH:, fs])))
                yield
            g, u = gu
            acts.append((_rb(g * jax.nn.sigmoid(g)) * u).astype(BF16))
        act = jnp.concatenate(acts, axis=1)
        for k in range(KD):
            ks = slice(k * 128, (k + 1) * 128)
            yacc[:, ks] += _nn(act, wd[pl.ds(f0, FC), ks])[:8]
            yield

    p1_block(NB - 1, (slots[0] + NB - 1) % 2, ffn=ffn_pieces(0))

    pr, pi = are8, aim8
    for _ in range(SEG.bit_length() - 1):
        pr, pi = pr * pr - pi * pi, 2.0 * pr * pi
    sub = jax.lax.broadcasted_iota(jnp.int32, (NSEG, P), 0)
    er = jnp.concatenate([hre[c] for c in range(NT)], axis=1)
    ei = jnp.concatenate([him[c] for c in range(NT)], axis=1)
    sh = 1
    while sh < NSEG:
        tr = jnp.where(sub >= sh, pltpu.roll(er, sh, 0), 0.0)
        ti = jnp.where(sub >= sh, pltpu.roll(ei, sh, 0), 0.0)
        er, ei = er + (pr * tr - pi * ti), ei + (pr * ti + pi * tr)
        pr, pi = pr * pr - pi * pi, 2.0 * pr * pi
        sh *= 2
    er = jnp.where(sub >= 1, pltpu.roll(er, 1, 0), 0.0)
    ei = jnp.where(sub >= 1, pltpu.roll(ei, 1, 0), 0.0)

    def scan(b, slot, c, init=None):
        cs = slice(c * 128, (c + 1) * 128)
        ar, ai, kr, ki = are8[:, cs], aim8[:, cs], kre8[:, cs], kim8[:, cs]
        nkr = -kr
        hr, hi = init or (hre[c], him[c])
        for j in range(0, J2, 4):
            ops = []
            for jj in (j, j + 2):
                h = []
                for step in (jj, jj + 1):
                    rows = pl.ds(pl.multiple_of(b * T2 + step * NSEG, NSEG), NSEG)
                    hr, hi = (ar * hr + bure[rows, cs]) - ai * hi, (ar * hi + buim[rows, cs]) + ai * hr
                    h += [kr * hr - ki * hi, nkr * hi - ki * hr]
                h11, h12, h21, h22 = h
                ops.append((h11 + h22, h21 + h22, h11, h22, h11 + h12, h21 - h11, h12 - h22))
            o = slice(j * NSEG // 2, j * NSEG // 2 + 16)
            for i in range(7):
                hb[slot, i, c, o, :] = jnp.concatenate([ops[0][i], ops[1][i]], 0).astype(BF16)
            if j + 4 == J2:
                hre[c] = hr
                him[c] = hi
            if (j + 4) % (J2 // 4) == 0:
                yield

    def p2_block(b, slot, last=False):
        ffn = iter(()) if last else itertools.chain(ffn_pieces(2 * b + 1), ffn_pieces(2 * b + 2))
        for n in range(DH // 128):
            ns = slice(n * 128, (n + 1) * 128)
            n2 = slice(DH + n * 128, DH + (n + 1) * 128)
            nxt = iter(()) if last else itertools.chain(
                scan(b + 1, 1 - slot, 2 * n), scan(b + 1, 1 - slot, 2 * n + 1))

            def prod(i, w):
                halves = []
                for half in range(2):
                    cc = range(half * (NT // 2), (half + 1) * (NT // 2))
                    lhs = jnp.concatenate([hb[slot, i, c] for c in cc], axis=1)
                    halves.append(_nt(lhs, w[:, half * (P // 2):(half + 1) * (P // 2)]))
                    next(ffn, None)
                next(nxt, None)
                return halves[0] + halves[1]

            def resid(ks):
                r = [_steps(xv[b * J + g, :, ks])
                     + xnf[pl.ds(pl.multiple_of(b * T2 + g * 16, 16), 16), ks].astype(F32) * dsk[:, ks]
                     for g in range(J)]
                return jnp.concatenate([v[:8] for v in r], 0), jnp.concatenate([v[8:] for v in r], 0)

            y11, y21 = resid(ns)
            y12, y22 = resid(n2)
            m = prod(0, ws.at[0, ns])
            y11, y22 = y11 + m, y22 + m
            m = prod(1, cre.at[ns])
            y21, y22 = y21 + m, y22 - m
            m = prod(2, ws.at[1, ns])
            y12, y22 = y12 + m, y22 + m
            m = prod(3, ws.at[2, ns])
            y11, y21 = y11 + m, y21 + m
            m = prod(4, cim.at[n2])
            y11, y12 = y11 - m, y12 + m
            y22 = y22 + prod(5, ws.at[3, ns])
            y11 = y11 + prod(6, ws.at[4, ns])
            next(nxt, None)
            for q, (ks, ya, yb) in enumerate(((ns, y11, y21), (n2, y12, y22))):
                slabs = [v[g * NSEG:(g + 1) * NSEG] for g in range(J) for v in (ya, yb)]
                if not last:
                    for j, v in enumerate(slabs):
                        stage[b * J2 + j, :, ks] = v
                    continue
                y = jnp.concatenate(slabs, axis=0)
                for s, j, yk in routed:
                    y = y + jnp.where(trow == (j - JL) * NSEG + s, yk[:, ks], 0.0)
                car[2 * n + q] = y
                for s in range(NSEG):
                    tail[s, :, ks] = car[2 * n + q, pl.ds(s, J2, stride=NSEG), :]
                if n >= 2:
                    cols = pl.ds(q * DH, 384) if n == 2 else ks
                    pltpu.make_async_copy(tail.at[:, :, cols],
                                          o_hbm.at[:, pl.ds(JL, J2), cols], sem_o.at[3]).start()
        if not last:
            start([o_copy(s, pl.multiple_of(b * J2, J2), J2, 0) for s in range(NSEG)])

    for c in range(NT):
        cs = slice(c * 128, (c + 1) * 128)
        for _ in scan(0, 0, c, (er[:, cs], ei[:, cs])):
            pass
    wait(w_copies[5:])
    jax.lax.fori_loop(0, NB2 - 1, lambda b, _: p2_block(b, b % 2), None)

    routed = [(t // SEG, t % SEG, yacc[k:k + 1, :] * jax.nn.sigmoid(jnp.full((1, D), m, F32)))
              for k, (t, m) in enumerate(((t1, m1), (t2, m2)))]
    trow = jax.lax.broadcasted_iota(jnp.int32, (T2, 128), 0)

    p2_block(NB2 - 1, (NB2 - 1) % 2, last=True)

    pltpu.make_async_copy(stage, stage, sem_o.at[0]).wait()
    sub8 = jax.lax.broadcasted_iota(jnp.int32, (NSEG, D), 0)
    for s, j, yk in routed:
        @pl.when(j < JL)
        def _():
            stage[j] = stage[j] + jnp.where(sub8 == s, yk, 0.0)
    (s1, j1, _), (s2, j2, _) = routed
    g1 = pl.multiple_of(j1 // 8 * 8, 8)
    g2 = pl.multiple_of(j2 // 8 * 8, 8)
    redo1 = g1 < JL
    redo2 = jnp.logical_and(g2 < JL, jnp.logical_or(g2 != g1, s2 != s1))
    pl.when(redo1)(lambda: o_copy(s1, g1, 8, 1).start())
    pl.when(redo2)(lambda: o_copy(s2, g2, 8, 2).start())
    pl.when(redo1)(lambda: o_copy(s1, g1, 8, 1).wait())
    pl.when(redo2)(lambda: o_copy(s2, g2, 8, 2).wait())
    pltpu.make_async_copy(tail, tail, sem_o.at[3]).wait()


@jax.jit
def pallas_parallel_sum__ssm_conv_s5__moe_arch_mod__prompt_kernel(
    A_x: jax.Array,
    A_Lambda_re: jax.Array,
    A_Lambda_im: jax.Array,
    A_B_re: jax.Array,
    A_B_im: jax.Array,
    A_C_re: jax.Array,
    A_C_im: jax.Array,
    A_log_dt: jax.Array,
    A_Dskip: jax.Array,
    B_x: jax.Array,
    B_w_r: jax.Array,
    B_w_gate: jax.Array,
    B_w_up: jax.Array,
    B_w_down: jax.Array,
):
    del B_x
    Bsz, S, D = A_x.shape
    P = A_B_re.shape[0]
    F = B_w_gate.shape[1]
    assert (Bsz, S, D, P, F) == (1, 2048, 1024, 1024, 3584)
    SEG, T = S // NSEG, NSEG * J
    hbm = pl.BlockSpec(memory_space=pl.ANY)
    vmem = pl.BlockSpec(memory_space=pltpu.VMEM)
    out = pl.pallas_call(
        _kernel,
        in_specs=[hbm, vmem, vmem, hbm, hbm, hbm, hbm, vmem, vmem, vmem, hbm, hbm, hbm],
        out_specs=hbm,
        out_shape=jax.ShapeDtypeStruct((NSEG, SEG, D), F32),
        scratch_shapes=[
            pltpu.VMEM((SEG // 2, NSEG, D), jnp.int32),
            pltpu.VMEM((P, D), BF16), pltpu.VMEM((P, D), BF16),
            pltpu.VMEM((D, P), BF16), pltpu.VMEM((D, P), BF16),
            pltpu.VMEM((D, F), BF16), pltpu.VMEM((D, F), BF16), pltpu.VMEM((F, D), BF16),
            pltpu.VMEM((S, P), F32), pltpu.VMEM((S, P), F32),
            pltpu.VMEM((P // 128, NSEG, 128), F32), pltpu.VMEM((P // 128, NSEG, 128), F32),
            pltpu.VMEM((2, NSEG, 128), F32), pltpu.VMEM((2, NSEG, 128), jnp.int32),
            pltpu.VMEM((D // 128, 2 * T, 128), F32),
            pltpu.VMEM((SEG - 2 * J, NSEG, D), F32),
            pltpu.VMEM((NSEG, 2 * J, D), F32),
            pltpu.VMEM((2, T, D), BF16),
            pltpu.VMEM((2, 7, P // 128, T, 128), BF16),
            pltpu.VMEM((S, D), BF16),
            pltpu.SMEM((1,), jnp.int32),
            pltpu.VMEM((5, D // 2, P), BF16),
            pltpu.VMEM((16, D), BF16), pltpu.VMEM((8, D), F32),
            pltpu.SemaphoreType.DMA((4,)),
            pltpu.SemaphoreType.DMA((2 * P // 128,)),
            pltpu.SemaphoreType.DMA((8,)),
            pltpu.SemaphoreType.DMA((4,)),
        ],
        compiler_params=pltpu.CompilerParams(vmem_limit_bytes=100 * 1024 * 1024),
    )(A_x.reshape(NSEG, SEG, D), A_Lambda_re, A_Lambda_im, A_B_re, A_B_im,
      A_C_re, A_C_im, A_log_dt, A_Dskip, B_w_r, B_w_gate, B_w_up, B_w_down)
    return out.reshape(Bsz, S, D)
```

```python
import itertools

import jax
import jax.numpy as jnp
import jax.experimental.pallas as pl
import jax.experimental.pallas.tpu as pltpu

F32 = jnp.float32
BF16 = jnp.bfloat16
NSEG = 8
J = 32


def _rb(v):
    return v.astype(BF16).astype(F32)


def _layernorm_rows(x):
    d = x.shape[-1]
    m = jnp.sum(x, axis=-1, keepdims=True) * (1.0 / d)
    mb = _rb(m)
    xc = x - mb
    v = jnp.sum(xc * xc, axis=-1, keepdims=True) * (1.0 / d) - (m - mb) * (m - mb)
    s = _rb(jnp.sqrt(_rb(_rb(v) + 1e-5)))
    return _rb(_rb(xc) / s)


def _steps(w):
    return jnp.concatenate([pltpu.bitcast(w << 16, F32), pltpu.bitcast(w & -65536, F32)], axis=0)


def _nt(a, b):
    return jax.lax.dot_general(a, b, (((1,), (1,)), ((), ())), preferred_element_type=F32)


def _nn(a, b):
    return jnp.dot(a, b, preferred_element_type=F32)


def _kernel(x_hbm, lre_ref, lim_ref, bre_hbm, bim_hbm, cre_hbm, cim_hbm, ldt_ref, dsk_ref,
            wr_ref, wg_hbm, wu_hbm, wd_hbm, o_hbm,
            xv, bre, bim, cre, cim, wg, wu, wd, bure, buim, hre, him, top, topi,
            car, stage, tail, xb, hb, xnf, slots, ws, xsel, yacc, sem_x, sem_b, sem_w, sem_o):
    S, D = xnf.shape
    P = bre.shape[0]
    F = wg.shape[1]
    KD, NT, DH = D // 128, P // 128, D // 2
    SEG = S // NSEG
    T, NB, JW = NSEG * J, SEG // J, J // 2
    J2 = 2 * J
    T2, NB2 = NSEG * J2, SEG // J2
    JL = SEG - J2
    FC = F // (2 * NB2 - 1)

    xw_hbm = x_hbm.bitcast(jnp.int32)

    class x_copy:
        def __init__(self, b, n=1):
            self.rows, self.sem = pl.ds(b * JW, n * JW), sem_x.at[b]

        def start(self):
            for s in range(NSEG):
                pltpu.make_async_copy(xw_hbm.at[s, self.rows, :], xv.at[self.rows, s, :], self.sem).start()

        def wait(self):
            pltpu.make_async_copy(xv.at[self.rows], xv.at[self.rows], self.sem).wait()

    def b_copies(c):
        rows = pl.ds(c * 128, 128)
        return [pltpu.make_async_copy(src.at[rows, :], dst.at[rows, :], sem_b.at[2 * c + k])
                for k, (src, dst) in enumerate(((bre_hbm, bre), (bim_hbm, bim)))]

    w_copies = [pltpu.make_async_copy(src, dst, sem_w.at[i]) for i, (src, dst) in enumerate(
        [(cre_hbm, cre), (cim_hbm, cim)]
        + [pair for f in (pl.ds(0, FC), pl.ds(FC, F - FC)) for pair in (
            (wg_hbm.at[:, f], wg.at[:, f]), (wu_hbm.at[:, f], wu.at[:, f]), (wd_hbm.at[f], wd.at[f]))])]

    def o_copy(s, j0, n, k):
        return pltpu.make_async_copy(
            stage.at[pl.ds(j0, n), s, :], o_hbm.at[s, pl.ds(j0, n), :], sem_o.at[k])

    def start(copies):
        for cp in copies:
            cp.start()

    def wait(copies):
        for cp in copies:
            cp.wait()

    x_copy(0).start()
    start(b_copies(0) + b_copies(1))

    row = lambda r: r[...].astype(F32).reshape(1, -1)
    lre, lim = row(lre_ref), row(lim_ref)
    dt = _rb(jnp.exp(row(ldt_ref)))
    mag = jnp.exp(dt * lre)
    are = mag * jnp.cos(dt * lim)
    aim = mag * jnp.sin(dt * lim)
    big = jnp.maximum(jnp.abs(lre), jnp.abs(lim))
    ure_, uim_ = lre / big, lim / big
    den = (ure_ * ure_ + uim_ * uim_) * big
    kre8 = jnp.broadcast_to(2.0 * ((are - 1.0) * ure_ + aim * uim_) / den, (NSEG, P))
    kim8 = jnp.broadcast_to(2.0 * (aim * ure_ - (are - 1.0) * uim_) / den, (NSEG, P))
    are8 = jnp.broadcast_to(are, (NSEG, P))
    aim8 = jnp.broadcast_to(aim, (NSEG, P))
    dsk = 1.0 + row(dsk_ref)
    wr = row(wr_ref)

    slots[0] = 0
    for c in range(NT):
        hre[c] = jnp.zeros((NSEG, 128), F32)
        him[c] = jnp.zeros((NSEG, 128), F32)
    yacc[...] = jnp.zeros_like(yacc)
    subd = jax.lax.broadcasted_iota(jnp.int32, (NSEG, 128), 0)
    top[0] = jnp.full((NSEG, 128), -jnp.inf, F32)
    top[1] = jnp.full((NSEG, 128), -jnp.inf, F32)
    topi[0] = subd * SEG
    topi[1] = subd * SEG + 1

    def norm(b, slot, g):
        rows = pl.ds(pl.multiple_of(b * T + g * 16, 16), 16)
        xn = _layernorm_rows(_steps(xv[b * JW + g]))
        xb[slot, g * 16:(g + 1) * 16, :] = xn.astype(BF16)
        xnf[rows, :] = xn.astype(BF16)
        r = jnp.broadcast_to(_rb(jnp.sum(xn * wr, axis=-1, keepdims=True)), (16, 128))
        b1, b2, i1, i2 = top[0], top[1], topi[0], topi[1]
        for j in range(2):
            rj = r[j * NSEG:(j + 1) * NSEG]
            tj = subd * SEG + (b * J + 2 * g + j)
            g1, g2 = rj > b1, rj > b2
            b2, i2 = jnp.where(g1, b1, jnp.where(g2, rj, b2)), jnp.where(g1, i1, jnp.where(g2, tj, i2))
            b1, i1 = jnp.where(g1, rj, b1), jnp.where(g1, tj, i1)
        top[0], top[1], topi[0], topi[1] = b1, b2, i1, i2

    def weight_sums(g):
        lo = pl.ds(pl.multiple_of(g * 16, 16), 16)
        up = pl.ds(pl.multiple_of(DH + g * 16, 16), 16)
        for cq in range(0, P, 256):
            cc = slice(cq, cq + 256)
            w11, w12 = cre[lo, cc].astype(F32), cre[up, cc].astype(F32)
            w21, w22 = cim[lo, cc].astype(F32), cim[up, cc].astype(F32)
            for q, v in enumerate((w11 + w22, w12 - w22, w21 - w11, w11 + w12, w21 + w22)):
                ws[q, lo, cc] = v.astype(BF16)

    def p1_block(b, slot, first=False, ffn=None, sums=False):
        r0 = pl.multiple_of(b * T, T)
        for c in range(NT):
            cs = slice(c * 128, (c + 1) * 128)
            if first:
                wait(b_copies(c))
                if c + 4 < NT:
                    start(b_copies(c + 4))
                elif c + 4 == NT:
                    x_copy(2).start()
                if c == 0:
                    x_copy(1).start()
                if c == NT // 2:
                    x_copy(1).wait()
            us = []
            for part, (w, bu) in enumerate(((bre, bure), (bim, buim))):
                u = _nt(xb[slot], w[cs, :])
                bu[pl.ds(r0, T), cs] = u
                us.append(u)
                g = 2 * c + part
                if ffn is not None and g >= 4:
                    next(ffn, None)
                    next(ffn, None)
                if ffn is not None or (first and g < NT):
                    xb[1 - slot, :16, :256] = jnp.zeros((16, 256), BF16)
                elif first:
                    norm(b + 1, 1 - slot, 2 * (g - NT))
                    norm(b + 1, 1 - slot, 2 * (g - NT) + 1)
                else:
                    norm(b + 1, 1 - slot, g)
                    if sums and part == 1:
                        weight_sums((b - 3) * NT + c)
            ure, uim = us
            ar, ai = are8[:, cs], aim8[:, cs]
            hr, hi = hre[c], him[c]
            for j in range(J):
                js = slice(j * NSEG, (j + 1) * NSEG)
                hr, hi = (ar * hr + ure[js]) - ai * hi, (ar * hi + uim[js]) + ai * hr
            hre[c] = hr
            him[c] = hi

    x_copy(0).wait()
    start(b_copies(2) + b_copies(3))
    for g in range(T // 16):
        norm(0, 0, g)
    p1_block(0, slots[0] % 2, first=True)
    x_rest = x_copy(3, NB - 3)
    x_rest.start()
    start(w_copies[:2])

    def p1_step(b, _):
        pl.when(b == 1)(x_copy(2).wait)

        @pl.when(b == 2)
        def _():
            x_rest.wait()
            start(w_copies[2:])

        p1_block(b, b % 2)

    jax.lax.fori_loop(1, 3, p1_step, None)
    wait(w_copies[:2])
    jax.lax.fori_loop(3, NB - 1, lambda b, _: p1_block(b, b % 2, sums=True), None)
    wait(w_copies[2:5])

    b1, b2, i1, i2 = top[0], top[1], topi[0], topi[1]
    m1 = jnp.max(b1)
    t1 = jnp.min(jnp.where(b1 == m1, i1, S))
    b1, i1 = jnp.where(i1 == t1, b2, b1), jnp.where(i1 == t1, i2, i1)
    m2 = jnp.max(b1)
    t2 = jnp.min(jnp.where(b1 == m2, i1, S))
    t1 = jnp.clip(t1, 0, S - 1)
    t2 = jnp.clip(t2, 0, S - 1)
    sub16 = jax.lax.broadcasted_iota(jnp.int32, (16, D), 0)

    def pick(t):
        s, j = t // SEG, t % SEG
        xn = _layernorm_rows(_steps(xv[j // 2]))
        return jnp.sum(jnp.where(sub16 == (j % 2) * NSEG + s, xn, 0.0), axis=0, keepdims=True)

    xs = jnp.where(sub16 == 0, pick(t1), jnp.where(sub16 == 1, pick(t2), 0.0))
    xsel[:, :DH] = xs[:, :DH].astype(BF16)
    xsel[:, DH:] = (-xs[:, DH:]).astype(BF16)

    def ffn_pieces(q):
        f0 = q * FC if isinstance(q, int) else pl.multiple_of(q * FC, FC)
        acts = []
        for n in range(FC // 128):
            fs = pl.ds(pl.multiple_of(f0 + n * 128, 128), 128)
            gu = []
            for w in (wg, wu):
                a = _nn(xsel[:, :DH], w[:DH, fs])
                yield
                gu.append(_rb(a - _nn(xsel[:, DH:], w[DH:, fs])))
                yield
            g, u = gu
            acts.append((_rb(g * jax.nn.sigmoid(g)) * u).astype(BF16))
        act = jnp.concatenate(acts, axis=1)
        for k in range(KD):
            ks = slice(k * 128, (k + 1) * 128)
            yacc[:, ks] += _nn(act, wd[pl.ds(f0, FC), ks])[:8]
            yield

    p1_block(NB - 1, (slots[0] + NB - 1) % 2, ffn=ffn_pieces(0))

    pr, pi = are8, aim8
    for _ in range(SEG.bit_length() - 1):
        pr, pi = pr * pr - pi * pi, 2.0 * pr * pi
    sub = jax.lax.broadcasted_iota(jnp.int32, (NSEG, P), 0)
    er = jnp.concatenate([hre[c] for c in range(NT)], axis=1)
    ei = jnp.concatenate([him[c] for c in range(NT)], axis=1)
    sh = 1
    while sh < NSEG:
        tr = jnp.where(sub >= sh, pltpu.roll(er, sh, 0), 0.0)
        ti = jnp.where(sub >= sh, pltpu.roll(ei, sh, 0), 0.0)
        er, ei = er + (pr * tr - pi * ti), ei + (pr * ti + pi * tr)
        pr, pi = pr * pr - pi * pi, 2.0 * pr * pi
        sh *= 2
    er = jnp.where(sub >= 1, pltpu.roll(er, 1, 0), 0.0)
    ei = jnp.where(sub >= 1, pltpu.roll(ei, 1, 0), 0.0)

    def scan(b, slot, c, init=None):
        cs = slice(c * 128, (c + 1) * 128)
        ar, ai, kr, ki = are8[:, cs], aim8[:, cs], kre8[:, cs], kim8[:, cs]
        nkr = -kr
        hr, hi = init or (hre[c], him[c])
        for j in range(0, J2, 4):
            ops = []
            for jj in (j, j + 2):
                h = []
                for step in (jj, jj + 1):
                    rows = pl.ds(pl.multiple_of(b * T2 + step * NSEG, NSEG), NSEG)
                    hr, hi = (ar * hr + bure[rows, cs]) - ai * hi, (ar * hi + buim[rows, cs]) + ai * hr
                    h += [kr * hr - ki * hi, nkr * hi - ki * hr]
                h11, h12, h21, h22 = h
                ops.append((h11 + h22, h21 + h22, h11, h22, h11 + h12, h21 - h11, h12 - h22))
            o = slice(j * NSEG // 2, j * NSEG // 2 + 16)
            for i in range(7):
                hb[slot, i, c, o, :] = jnp.concatenate([ops[0][i], ops[1][i]], 0).astype(BF16)
            if j + 4 == J2:
                hre[c] = hr
                him[c] = hi
            if (j + 4) % (J2 // 4) == 0:
                yield

    def p2_block(b, slot, last=False):
        ffn = iter(()) if last else itertools.chain(ffn_pieces(2 * b + 1), ffn_pieces(2 * b + 2))
        for n in range(DH // 128):
            ns = slice(n * 128, (n + 1) * 128)
            n2 = slice(DH + n * 128, DH + (n + 1) * 128)
            nxt = iter(()) if last else itertools.chain(
                scan(b + 1, 1 - slot, 2 * n), scan(b + 1, 1 - slot, 2 * n + 1))

            def prod(i, w):
                halves = []
                for half in range(2):
                    cc = range(half * (NT // 2), (half + 1) * (NT // 2))
                    lhs = jnp.concatenate([hb[slot, i, c] for c in cc], axis=1)
                    halves.append(_nt(lhs, w[:, half * (P // 2):(half + 1) * (P // 2)]))
                    next(ffn, None)
                next(nxt, None)
                return halves[0] + halves[1]

            def resid(ks):
                r = [_steps(xv[b * J + g, :, ks])
                     + xnf[pl.ds(pl.multiple_of(b * T2 + g * 16, 16), 16), ks].astype(F32) * dsk[:, ks]
                     for g in range(J)]
                return jnp.concatenate([v[:8] for v in r], 0), jnp.concatenate([v[8:] for v in r], 0)

            y11, y21 = resid(ns)
            y12, y22 = resid(n2)
            m = prod(0, ws.at[0, ns])
            y11, y22 = y11 + m, y22 + m
            m = prod(1, cre.at[ns])
            y21, y22 = y21 + m, y22 - m
            m = prod(2, ws.at[1, ns])
            y12, y22 = y12 + m, y22 + m
            m = prod(3, ws.at[2, ns])
            y11, y21 = y11 + m, y21 + m
            m = prod(4, cim.at[n2])
            y11, y12 = y11 - m, y12 + m
            y22 = y22 + prod(5, ws.at[3, ns])
            y11 = y11 + prod(6, ws.at[4, ns])
            next(nxt, None)
            for q, (ks, ya, yb) in enumerate(((ns, y11, y21), (n2, y12, y22))):
                slabs = [v[g * NSEG:(g + 1) * NSEG] for g in range(J) for v in (ya, yb)]
                if not last:
                    for j, v in enumerate(slabs):
                        stage[b * J2 + j, :, ks] = v
                    continue
                y = jnp.concatenate(slabs, axis=0)
                for s, j, yk in routed:
                    y = y + jnp.where(trow == (j - JL) * NSEG + s, yk[:, ks], 0.0)
                car[2 * n + q] = y
                for s in range(NSEG):
                    tail[s, :, ks] = car[2 * n + q, pl.ds(s, J2, stride=NSEG), :]
                if n >= 2:
                    cols = pl.ds(q * DH, 384) if n == 2 else ks
                    pltpu.make_async_copy(tail.at[:, :, cols],
                                          o_hbm.at[:, pl.ds(JL, J2), cols], sem_o.at[3]).start()
        if not last:
            start([o_copy(s, pl.multiple_of(b * J2, J2), J2, 0) for s in range(NSEG)])

    for c in range(NT):
        cs = slice(c * 128, (c + 1) * 128)
        for _ in scan(0, 0, c, (er[:, cs], ei[:, cs])):
            pass
    wait(w_copies[5:])
    jax.lax.fori_loop(0, NB2 - 1, lambda b, _: p2_block(b, b % 2), None)

    routed = [(t // SEG, t % SEG, yacc[k:k + 1, :] * jax.nn.sigmoid(jnp.full((1, D), m, F32)))
              for k, (t, m) in enumerate(((t1, m1), (t2, m2)))]
    trow = jax.lax.broadcasted_iota(jnp.int32, (T2, 128), 0)

    p2_block(NB2 - 1, (NB2 - 1) % 2, last=True)

    pltpu.make_async_copy(stage, stage, sem_o.at[0]).wait()
    sub8 = jax.lax.broadcasted_iota(jnp.int32, (NSEG, D), 0)
    for s, j, yk in routed:
        @pl.when(j < JL)
        def _():
            stage[j] = stage[j] + jnp.where(sub8 == s, yk, 0.0)
    (s1, j1, _), (s2, j2, _) = routed
    g1 = pl.multiple_of(j1 // 8 * 8, 8)
    g2 = pl.multiple_of(j2 // 8 * 8, 8)
    redo1 = g1 < JL
    redo2 = jnp.logical_and(g2 < JL, jnp.logical_or(g2 != g1, s2 != s1))
    pl.when(redo1)(lambda: o_copy(s1, g1, 8, 1).start())
    pl.when(redo2)(lambda: o_copy(s2, g2, 8, 2).start())
    pl.when(redo1)(lambda: o_copy(s1, g1, 8, 1).wait())
    pl.when(redo2)(lambda: o_copy(s2, g2, 8, 2).wait())
    pltpu.make_async_copy(tail, tail, sem_o.at[3]).wait()


@jax.jit
def pallas_parallel_sum__ssm_conv_s5__moe_arch_mod__prompt_kernel(
    A_x: jax.Array,
    A_Lambda_re: jax.Array,
    A_Lambda_im: jax.Array,
    A_B_re: jax.Array,
    A_B_im: jax.Array,
    A_C_re: jax.Array,
    A_C_im: jax.Array,
    A_log_dt: jax.Array,
    A_Dskip: jax.Array,
    B_x: jax.Array,
    B_w_r: jax.Array,
    B_w_gate: jax.Array,
    B_w_up: jax.Array,
    B_w_down: jax.Array,
):
    del B_x
    Bsz, S, D = A_x.shape
    P = A_B_re.shape[0]
    F = B_w_gate.shape[1]
    assert (Bsz, S, D, P, F) == (1, 2048, 1024, 1024, 3584)
    SEG, T = S // NSEG, NSEG * J
    hbm = pl.BlockSpec(memory_space=pl.ANY)
    vmem = pl.BlockSpec(memory_space=pltpu.VMEM)
    out = pl.pallas_call(
        _kernel,
        in_specs=[hbm, vmem, vmem, hbm, hbm, hbm, hbm, vmem, vmem, vmem, hbm, hbm, hbm],
        out_specs=hbm,
        out_shape=jax.ShapeDtypeStruct((NSEG, SEG, D), F32),
        scratch_shapes=[
            pltpu.VMEM((SEG // 2, NSEG, D), jnp.int32),
            pltpu.VMEM((P, D), BF16), pltpu.VMEM((P, D), BF16),
            pltpu.VMEM((D, P), BF16), pltpu.VMEM((D, P), BF16),
            pltpu.VMEM((D, F), BF16), pltpu.VMEM((D, F), BF16), pltpu.VMEM((F, D), BF16),
            pltpu.VMEM((S, P), F32), pltpu.VMEM((S, P), F32),
            pltpu.VMEM((P // 128, NSEG, 128), F32), pltpu.VMEM((P // 128, NSEG, 128), F32),
            pltpu.VMEM((2, NSEG, 128), F32), pltpu.VMEM((2, NSEG, 128), jnp.int32),
            pltpu.VMEM((D // 128, 2 * T, 128), F32),
            pltpu.VMEM((SEG - 2 * J, NSEG, D), F32),
            pltpu.VMEM((NSEG, 2 * J, D), F32),
            pltpu.VMEM((2, T, D), BF16),
            pltpu.VMEM((2, 7, P // 128, T, 128), BF16),
            pltpu.VMEM((S, D), BF16),
            pltpu.SMEM((1,), jnp.int32),
            pltpu.VMEM((5, D // 2, P), BF16),
            pltpu.VMEM((16, D), BF16), pltpu.VMEM((8, D), F32),
            pltpu.SemaphoreType.DMA((4,)),
            pltpu.SemaphoreType.DMA((2 * P // 128,)),
            pltpu.SemaphoreType.DMA((8,)),
            pltpu.SemaphoreType.DMA((4,)),
        ],
        compiler_params=pltpu.CompilerParams(vmem_limit_bytes=100 * 1024 * 1024),
    )(A_x.reshape(NSEG, SEG, D), A_Lambda_re, A_Lambda_im, A_B_re, A_B_im,
      A_C_re, A_C_im, A_log_dt, A_Dskip, B_w_r, B_w_gate, B_w_up, B_w_down)
    return out.reshape(Bsz, S, D)
```
